```python
import os as _os
_os.environ.setdefault("JAX_PLATFORMS", "cpu")
import jax
import jax.numpy as jnp

def _softmax(x, axis=-1):
    return jax.nn.softmax(x, axis=axis)
def _gelu(x):
    return jax.nn.gelu(x, approximate=True)
def _silu(x):
    return jax.nn.silu(x)
def _sigmoid(x):
    return jax.nn.sigmoid(x)
def _layernorm(x, axis=-1, eps=1e-5):
    m = jnp.mean(x, axis=axis, keepdims=True)
    v = jnp.var(x, axis=axis, keepdims=True)
    return (x - m) / jnp.sqrt(v + eps)
def _scatter_add(tgt, idx, src, axis=0):
    return tgt.at[idx].add(src)
def _segment_sum(src, seg, n):
    return jax.ops.segment_sum(src, seg, n)
class _Rng:
    def __init__(self, key):
        self._k = key
    def _next(self):
        self._k, sub = jax.random.split(self._k)
        return sub
    def normal(self, shape):
        return jax.random.normal(self._next(), shape, dtype=jnp.bfloat16)
    def randint(self, lo, hi, shape):
        return jax.random.randint(self._next(), shape, lo, hi, dtype=jnp.int32)
    def uniform(self, shape, lo=0.0, hi=1.0):
        return jax.random.uniform(self._next(), shape, jnp.bfloat16, lo, hi)
    def permutation(self, n):
        return jax.random.permutation(self._next(), n)


kernel_name = 'interleave_layers__sliding_block_cached__mixer_channel_mlp__decode'

def setup_inputs():
    _rng = _Rng(jax.random.key(int.from_bytes(__import__("os").urandom(4), "little")))
    _w = (lambda a: (lambda t: t.astype(jnp.bfloat16) if jnp.issubdtype(t.dtype, jnp.floating) else t)(jnp.asarray(a)))
    def _A_setup():
        B, Sq, D = 8, 1, 640
        Hq, Hkv, Sk, Dh = 32, 32, 4096, 128
        assert Hq % Hkv == 0, (Hq, Hkv)
        return {
            "x": _w((lambda *s: _rng.normal(s) * 0.05)(B, Sq, D)),
            "k_cache": _w((lambda *s: _rng.normal(s) * 1.6)(B, Hkv, Sk, Dh)),
            "v_cache": _w((lambda *s: _rng.normal(s) * 0.8)(B, Hkv, Sk, Dh)),
            "wq": _w((lambda *s: _rng.normal(s) * 1.6)(D, Hq * Dh) * (D ** -0.5)),
            "wo": _w((lambda *s: _rng.normal(s) * 0.8)(Hq * Dh, D) * ((Hq * Dh) ** -0.5)),
        }
    _A_in = _A_setup()

    def _B_setup():
        B, S, D, F = 8, 1, 640, 1728
        return {
            "x": _w((lambda *s: _rng.normal(s) * 0.05)(B, S, D)),
            "w1": _w((lambda *s: _rng.normal(s) * 0.4)(D, F) * (D ** -0.5)),
            "b1": _w((lambda *s: _rng.normal(s) * 0.4)(F)),
            "w2": _w((lambda *s: _rng.normal(s) * 0.4)(F, D) * (F ** -0.5)),
            "b2": _w((lambda *s: _rng.normal(s) * 0.2)(D)),
        }
    _B_in = _B_setup()

    return {
        "A_x": _A_in["x"],
        "A_k_cache": _A_in["k_cache"],
        "A_v_cache": _A_in["v_cache"],
        "A_wq": _A_in["wq"],
        "A_wo": _A_in["wo"],
        "B_x": _B_in["x"],
        "B_w1": _B_in["w1"],
        "B_b1": _B_in["b1"],
        "B_w2": _B_in["w2"],
        "B_b2": _B_in["b2"],
    }

def reference(A_x, A_k_cache, A_v_cache, A_wq, A_wo, B_x, B_w1, B_b1, B_w2, B_b2):
    def _A_ref(x, k_cache, v_cache, wq, wo):
        B, Sq, D = x.shape
        Hq, Dh = 32, 128
        Hkv, Sk = k_cache.shape[1], k_cache.shape[2]
        W = min(4096, max(256, Sk // 4))
        rep = Hq // Hkv
        q = (lambda x, *d: x.transpose(*d))((x @ wq).reshape(B, Sq, Hq, Dh), 0, 2, 1, 3)
        k = jnp.repeat(k_cache[:, :, Sk - W:, :], rep, axis=1)
        v = jnp.repeat(v_cache[:, :, Sk - W:, :], rep, axis=1)
        scores = jnp.einsum("bhqd,bhkd->bhqk", q, k) * (Dh ** -0.5)
        p = _softmax(scores, axis=-1)
        o = jnp.einsum("bhqk,bhkd->bhqd", p, v)
        return (lambda x, *d: x.transpose(*d))(o, 0, 2, 1, 3).reshape(B, Sq, Hq * Dh) @ wo

    def _B_ref(x, w1, b1, w2, b2):
        y = _layernorm(x, axis=-1)
        h = _gelu(jnp.einsum("bsd,df->bsf", y, w1) + b1)
        return jnp.einsum("bsf,fd->bsd", h, w2) + b2

    x = A_x
    x = x + _A_ref(_layernorm(x, axis=-1), A_k_cache, A_v_cache, A_wq, A_wo)
    x = x + _B_ref(_layernorm(x, axis=-1), B_w1, B_b1, B_w2, B_b2)
    x = x + _A_ref(_layernorm(x, axis=-1), A_k_cache, A_v_cache, A_wq, A_wo)
    x = x + _B_ref(_layernorm(x, axis=-1), B_w1, B_b1, B_w2, B_b2)
    return x
```

```python
import functools

import jax
import jax.numpy as jnp
from jax import lax
from jax.experimental import pallas as pl
from jax.experimental.pallas import tpu as pltpu

B, D, H, DH, SK, F = 8, 640, 32, 128, 4096, 1728
W = min(4096, max(256, SK // 4))
FP = 1792
G = 8
NG = H // G
ROWS = 128
NT = (((1,), (1,)), ((), ()))
LOG2E = 1.4426950408889634
F32, BF16 = jnp.float32, jnp.bfloat16


def build(prio="0111", compute=True, bounds=False):
    def kern(x_hbm, k_hbm, v_hbm, wq_hbm, wo_hbm, w1t_hbm, b1_hbm, w2_hbm, b2_hbm,
             o_ref,
             kbuf, vbuf, wq, wo, w1t, w1, w2, xb, b1v, b2v,
             xs, q1, b1s, b2s, pscr, lscr, res, sems):
        S_K, S_V01, S_V2, S_V3, S_SM, S_WQ, S_W1, S_WO = range(8)
        cnt = [0]

        def nxt_prio():
            p = int(prio[cnt[0] % len(prio)])
            cnt[0] += 1
            return p

        def kv_quarter(src, dst, b, g, quarter, sem):
            slot = b % 2
            for s in (2 * quarter, 2 * quarter + 1):
                for j in range(G):
                    h = g * G + j
                    pltpu.make_async_copy(
                        src.at[b, h, pl.ds(SK - W + s * ROWS, ROWS), :],
                        dst.at[slot, h, pl.ds(s * ROWS, ROWS), :],
                        sems.at[sem]).start(priority=nxt_prio())

        def vsem(g):
            return (S_V01, S_V01, S_V2, S_V3)[g]

        def issue_k(b, g, quarter):
            kv_quarter(k_hbm, kbuf, b, g, quarter, S_K)

        def issue_v(b, g, quarter):
            kv_quarter(v_hbm, vbuf, b, g, quarter, vsem(g))

        def wait_full(ref, sem):
            pltpu.make_async_copy(ref, ref, sems.at[sem]).wait()

        def rows_copy(src, dst, n, step, sem):
            starts = list(range(0, n, step))
            k = 8
            per = -(-len(starts) // k)
            order = [starts[i] for r in range(per) for i in range(r, len(starts), per)]
            for r0 in order:
                sz = min(step, n - r0)
                pltpu.make_async_copy(src.at[pl.ds(r0, sz), :], dst.at[pl.ds(r0, sz), :],
                                      sems.at[sem]).start(priority=nxt_prio())

        row = lax.broadcasted_iota(jnp.int32, (8, 128), 0)

        def layernorm(x):
            m = jnp.mean(x, axis=-1, keepdims=True)
            d = x - m
            v = jnp.mean(d * d, axis=-1, keepdims=True)
            return d * lax.rsqrt(v + 1e-5)

        def gelu(x):
            c = 0.7978845608028654
            return 0.5 * x * (1.0 + jnp.tanh(c * (x + 0.044715 * (x * x * x))))

        def mlp(x, tick):
            y = layernorm(x).astype(BF16)
            h = jnp.dot(y, w1[...], preferred_element_type=F32) + b1s[...]
            tick()
            h = gelu(h).astype(BF16)
            return x + jnp.dot(h, w2[...], preferred_element_type=F32) + b2s[...]

        def scores(slot, g, q_of, tick):
            rowk = lax.broadcasted_iota(jnp.int32, (8, W), 0)
            s = None
            for j in range(G):
                sj = lax.dot_general(q_of(j), kbuf[slot, g * G + j], NT, preferred_element_type=F32)
                s = sj if s is None else jnp.where(rowk == j, sj, s)
                if j == G // 2 - 1:
                    tick()
            m = jnp.max(s, axis=-1, keepdims=True)
            p = jnp.exp2((s - m) * (DH ** -0.5 * LOG2E))
            l = jnp.sum(p, axis=-1, keepdims=True)
            return p, 1.0 / l

        def pv_wo(slot, g, p, inv, tick):
            pb = p.astype(BF16)
            parts = []
            for j in range(G):
                oj = jnp.dot(pb, vbuf[slot, g * G + j], preferred_element_type=F32)
                parts.append(jnp.where(row == j, oj * inv, 0.0))
            tick()
            lhs = jnp.concatenate(parts, axis=1).astype(BF16)
            return jnp.dot(lhs, wo[g * G * DH:(g + 1) * G * DH, :], preferred_element_type=F32)

        sm = [pltpu.make_async_copy(x_hbm, xb, sems.at[S_SM]),
              pltpu.make_async_copy(b1_hbm, b1v, sems.at[S_SM]),
              pltpu.make_async_copy(b2_hbm, b2v, sems.at[S_SM])]
        for r in range(0, D // 16, 1):
            for c in range(4):
                r0 = ((r % 2) * (D // 32) + r // 2) * 16
                pltpu.make_async_copy(wq_hbm.at[pl.ds(r0, 16), pl.ds(c * 1024, 1024)],
                                      wq.at[pl.ds(r0, 16), pl.ds(c * 1024, 1024)],
                                      sems.at[S_WQ]).start(priority=nxt_prio())
            if r == 3:
                for c in sm:
                    c.start()
        rows_copy(w1t_hbm, w1t, F, 32, S_W1)
        w1t[F:FP, :] = jnp.zeros((FP - F, D), BF16)
        w2[F:FP, :] = jnp.zeros((FP - F, D), BF16)
        rows_copy(wo_hbm, wo, H * DH, 32, S_WO)
        for c in sm:
            c.wait()
        x0 = xb[...].astype(F32)
        for i in range(B):
            xs[i] = jnp.broadcast_to(x0[i:i + 1, :], (8, D))
        b1s[...] = jnp.zeros((8, FP), F32)
        b1s[:, 0:F] = jnp.broadcast_to(b1v[...].astype(F32).reshape(1, F), (8, F))
        b2s[...] = jnp.broadcast_to(b2v[...].astype(F32).reshape(1, D), (8, D))
        res[...] = jnp.zeros((8, D), F32)
        wait_full(wq, S_WQ)
        qa = jnp.dot(layernorm(x0).astype(BF16), wq[...], preferred_element_type=F32)
        for i in range(B):
            q1[i] = jnp.broadcast_to(qa[i:i + 1, :], (8, H * DH))
        rows_copy(w2_hbm, w2, F, 32, S_WO)
        wait_full(w1t.at[pl.ds(0, F), :], S_W1)
        for g in range(NG):
            for qt in range(4):
                issue_k(0, g, qt)
                i = g * 4 + qt
                if i < FP // 128:
                    w1[:, i * 128:(i + 1) * 128] = w1t[i * 128:(i + 1) * 128, :].T
        for g in range(2):
            for qt in range(4):
                issue_v(0, g, qt)
        wait_full(wo, S_WO)
        wait_full(w2.at[pl.ds(0, F), :], S_WO)

        def body(b, carry):
            slot = b % 2
            plan = ([functools.partial(issue_v, b, g, qt) for g in (2, 3) for qt in range(4)])

            def later(f, g, qt):
                @pl.when(b + 1 < B)
                def _():
                    f(b + 1, g, qt)
            plan += [functools.partial(later, issue_k, g, qt) for g in range(NG) for qt in range(4)]
            plan += [functools.partial(later, issue_v, g, qt) for g in range(2) for qt in range(4)]
            pos = [0]

            def tick(n=1):
                for _ in range(n):
                    plan[pos[0]]()
                    pos[0] += 1

            if not compute:
                tick(4)
                wait_full(kbuf.at[slot], S_K)
                tick(4)
                wait_full(vbuf.at[slot, pl.ds(0, 2 * G)], S_V01)
                tick(4)
                wait_full(vbuf.at[slot, pl.ds(2 * G, G)], S_V2)
                tick(4)
                wait_full(vbuf.at[slot, pl.ds(3 * G, G)], S_V3)
                tick(16)
                return carry

            wait_full(kbuf.at[slot], S_K)
            for g in range(NG):
                tick()

                def q_of(j, g=g):
                    h = g * G + j
                    return q1[b, :, h * DH:(h + 1) * DH].astype(BF16)
                p, inv = scores(slot, g, q_of, tick)
                pscr[g] = p
                lscr[g] = jnp.broadcast_to(inv, (8, 128))
            assert pos[0] == 8
            wait_full(vbuf.at[slot, pl.ds(0, 2 * G)], S_V01)
            acc = pv_wo(slot, 0, pscr[0], lscr[0], tick)
            tick()
            acc += pv_wo(slot, 1, pscr[1], lscr[1], tick)
            tick()
            wait_full(vbuf.at[slot, pl.ds(2 * G, G)], S_V2)
            acc += pv_wo(slot, 2, pscr[2], lscr[2], tick)
            wait_full(vbuf.at[slot, pl.ds(3 * G, G)], S_V3)
            tick()
            acc += pv_wo(slot, 3, pscr[3], lscr[3], tick)
            x = xs[b]
            x = x + jnp.sum(acc, axis=0, keepdims=True)
            tick()
            x = mlp(x, tick)
            assert pos[0] == 17
            y = layernorm(x).astype(BF16)
            acc = None
            for g in range(NG):
                tick()
                q = jnp.dot(y, wq[:, g * G * DH:(g + 1) * G * DH], preferred_element_type=F32).astype(BF16)
                p, inv = scores(slot, g, lambda j: q[:, j * DH:(j + 1) * DH], tick)
                a = pv_wo(slot, g, p, inv, tick)
                acc = a if acc is None else acc + a
            x = x + jnp.sum(acc, axis=0, keepdims=True)
            tick()
            x = mlp(x, tick)
            tick()
            assert pos[0] == 32
            rowd = lax.broadcasted_iota(jnp.int32, (8, D), 0)
            res[...] = jnp.where(rowd == b, x, res[...])
            return carry

        lax.fori_loop(0, B, body, 0)
        o_ref[...] = res[...].astype(BF16)

    hbm = pl.BlockSpec(memory_space=pltpu.HBM)
    call = pl.pallas_call(
        kern,
        out_shape=jax.ShapeDtypeStruct((B, D), BF16),
        in_specs=[hbm] * 9,
        out_specs=pl.BlockSpec(memory_space=pltpu.VMEM),
        scratch_shapes=[
            pltpu.VMEM((2, H, W, DH), BF16), pltpu.VMEM((2, H, W, DH), BF16),
            pltpu.VMEM((D, H * DH), BF16), pltpu.VMEM((H * DH, D), BF16),
            pltpu.VMEM((FP, D), BF16), pltpu.VMEM((D, FP), BF16), pltpu.VMEM((FP, D), BF16),
            pltpu.VMEM((B, D), BF16), pltpu.VMEM((F,), BF16), pltpu.VMEM((D,), BF16),
            pltpu.VMEM((B, 8, D), F32), pltpu.VMEM((B, 8, H * DH), F32),
            pltpu.VMEM((8, FP), F32), pltpu.VMEM((8, D), F32),
            pltpu.VMEM((NG, 8, W), F32), pltpu.VMEM((NG, 8, 128), F32),
            pltpu.VMEM((B, D), F32),
            pltpu.SemaphoreType.DMA((8,)),
        ],
        compiler_params=pltpu.CompilerParams(
            vmem_limit_bytes=100 * 1024 * 1024, disable_bounds_checks=not bounds),
    )

    return call


@jax.jit
def pallas_interleave_layers__sliding_block_cached__mixer_channel_mlp__decode_kernel(
    A_x, A_k_cache, A_v_cache, A_wq, A_wo, B_x, B_w1, B_b1, B_w2, B_b2):
    out = build()(A_x.reshape(B, D), A_k_cache, A_v_cache, A_wq, A_wo, B_w1.T, B_b1, B_w2, B_b2)
    return out.reshape(B, 1, D)
```

```python
import functools

import jax
import jax.numpy as jnp
from jax import lax
from jax.experimental import pallas as pl
from jax.experimental.pallas import tpu as pltpu

B, D, H, DH, SK, F = 8, 640, 32, 128, 4096, 1728
W = min(4096, max(256, SK // 4))
G = 8
NG = H // G
NC = D // 128
NKT = W // 128
NF = -(-F // 128)
ROWS = 128
NT = (((1,), (1,)), ((), ()))
LOG2E = 1.4426950408889634
F32, BF16, U32 = jnp.float32, jnp.bfloat16, jnp.uint32


def _interleave(*streams):
    t = [0.0] * len(streams)
    live = list(range(len(streams)))
    while live:
        for i in sorted(live, key=lambda i: t[i]):
            try:
                c = next(streams[i])
            except StopIteration:
                live.remove(i)
                break
            if c is not None:
                t[i] += c
                break
            t[i] = max(t[i], min([t[j] for j in live if j != i], default=t[i]))
        else:
            raise RuntimeError("deadlock")


def _tree(op, xs):
    xs = list(xs)
    while len(xs) > 1:
        xs = [op(xs[i], xs[i + 1]) if i + 1 < len(xs) else xs[i] for i in range(0, len(xs), 2)]
    return xs[0]


def _spread(items, k):
    per = -(-len(items) // k)
    return [items[i] for r in range(per) for i in range(r, len(items), per)]


def build(prio="0111", compute=True, tail=True, nfm=9, dchunk=4, fchunk=4, mchain=16, vchain=4, vcost=1.15, mcost=1.07,
          chain=112, fcost=1.0, fskew=0, last=(8, 4, 2, 2), wrows=16, flags=None, lastprio=None, pre_k=4, nb=B - 1, dma=True, ST=9, vpre=5):
    MG, VG = (0, 1), (2, 3)
    FV = F - nfm * 128

    def kern(x_hbm, k_hbm, v_hbm, wq_hbm, wo_hbm, w1t_hbm, b1_hbm, w2_hbm, b2_hbm,
             o_ref,
             kv, wq, wo, w1t, w2, xb, b1v, b2v,
             wqm, wom, w1m, w2m, wqf, wof, w1f, w2f, b1c, ktm, ktf, vtf,
             xs, q1, b1s, b2s, pscr, lscr, res, zero, sems):
        S_K, S_VHI, S_VLO = 0, 1, 2
        S_SM, S_WQ, S_W1, S_WO = 2, 3, 4, 5
        cnt = [0]

        def start(src, dst, sem, pr=None):
            p = int(prio[cnt[0] % len(prio)]) if pr is None else pr
            cnt[0] += 1
            pltpu.make_async_copy(src, dst, sems.at[sem]).start(priority=p)

        def wait(ref, sem):
            if not dma and sem <= S_VLO:
                return
            pltpu.make_async_copy(ref, ref, sems.at[sem]).wait()

        def kv_copy(w, b, h, s, sem, pr=None):
            if dma:
                r0 = s * ROWS if isinstance(s, int) else pl.multiple_of(s * ROWS, ROWS)
                start((k_hbm, v_hbm)[w].at[b, h, pl.ds(SK - W + r0, ROWS), :],
                      kv.at[b % 2, w, h, pl.ds(r0, ROWS), :], sem, pr)

        def kv_ticks(w, b, heads, sem, pr=None):
            items = [(h, s) for s in range(W // ROWS) for h in heads]

            def tick(part):
                for i, (h, s) in enumerate(part):
                    kv_copy(w, b, h, s, sem, None if pr is None else int(pr[i % len(pr)]))
            return [functools.partial(tick, items[i:i + 16]) for i in range(0, len(items), 16)]

        class Plan:
            def __init__(self, ticks):
                self.ticks, self.pos = ticks, 0

            def __call__(self, n=1):
                for _ in range(min(n, len(self.ticks) - self.pos)):
                    self.ticks[self.pos]()
                    self.pos += 1

        row = lax.broadcasted_iota(jnp.int32, (8, 128), 0)
        bf = lambda u: pltpu.bitcast(u, BF16)
        ldk = lambda slot, h: bf(kv.bitcast(U32)[slot, 0, h])
        ldv = lambda slot, h: bf(kv.bitcast(U32)[slot, 1, h])
        mm = functools.partial(jnp.dot, preferred_element_type=F32)
        add = lambda a, b: a + b

        def cols(x):
            return [x[:, c * 128:(c + 1) * 128] for c in range(x.shape[1] // 128)]

        def lanesum(a):
            return jnp.broadcast_to(jnp.sum(a, axis=1, keepdims=True), (8, 128))

        def center(x):
            d = x - jnp.mean(x, axis=-1, keepdims=True)
            v = jnp.mean(d * d, axis=-1, keepdims=True)
            return d, jnp.broadcast_to(lax.rsqrt(v + 1e-5), (8, 128))

        def gelu(x):
            c = 0.7978845608028654
            return 0.5 * x * (1.0 + jnp.tanh(x * (c + (c * 0.044715) * (x * x))))

        def softmax(s, scale):
            m = jnp.broadcast_to(jnp.max(_tree(jnp.maximum, s), axis=1, keepdims=True), (8, 128))
            p = [jnp.exp2((t - m) * scale) for t in s]
            return p, 1.0 / lanesum(_tree(add, p))

        def scores(slot, g, q_of, scale, tick):
            s = None
            for j in range(G):
                sj = cols(lax.dot_general(q_of(j), ldk(slot, g * G + j), NT, preferred_element_type=F32))
                s = sj if s is None else [jnp.where(row == j, a, b) for a, b in zip(sj, s)]
                if j == G // 2 - 1:
                    tick()
            return softmax(s, scale)

        def pv_wo(slot, heads, p, inv, acc):
            pb = jnp.concatenate(p, axis=1).astype(BF16)
            parts = [jnp.where(row == h % G, mm(pb, ldv(slot, h)) * inv, 0.0) for h in heads]
            lhs = jnp.concatenate(parts, axis=1).astype(BF16)
            rs = slice(heads[0] * DH // 2, (heads[-1] + 1) * DH // 2)
            out = [mm(lhs, bf(wom[c, rs, :])) for c in range(NC)]
            return out if acc is None else [a + o for a, o in zip(acc, out)]

        def residual(x, acc):
            return x + jnp.sum(jnp.concatenate(acc, axis=1), axis=0, keepdims=True)

        def mlp(x, tick):
            y, r = center(x)
            yb = y.astype(BF16)
            h = [gelu(mm(yb, bf(w1m[i])) * r + b1s[:, i * 128:(i + 1) * 128]) for i in range(NF)]
            tick()
            hb = jnp.concatenate(h, axis=1).astype(BF16)
            return x + b2s[...] + jnp.concatenate([mm(hb, bf(w2m[c])) for c in range(NC)], axis=1)

        def mlp_dual(x, never):
            y, r = center(x)
            yb, yc = y.astype(BF16), cols(y)
            st = {}

            def mxu():
                hs = []
                for i in range(nfm):
                    hs.append(gelu(mm(yb, bf(w1m[i])) * r + b1s[:, i * 128:(i + 1) * 128]))
                    yield 40 * mcost
                hb = jnp.concatenate(hs, axis=1).astype(BF16)
                st["m"] = []
                for c in range(NC):
                    st["m"].append(mm(hb, bf(w2m[c, 0:nfm * 64, :])))
                    yield nfm * 8 * mcost

            def vpu():
                acc = [None] * NC
                pend = []

                def second(ch, hv):
                    for fg, h in zip(ch, hv):
                        for c in range(NC):
                            pr = w2f[c, fg * 8:fg * 8 + 8, :] * h
                            acc[c] = pr if acc[c] is None else acc[c] + pr
                for i0 in range(0, FV // 8, fchunk):
                    ch = range(i0, min(i0 + fchunk, FV // 8))
                    hv = [lanesum(_tree(add, [w1f[c, fg * 8:fg * 8 + 8, :] * yc[c] for c in range(NC)])) for fg in ch]
                    yield len(hv) * 9 / 4 * fcost
                    hv = [gelu(h * r + b1c[fg * 8:fg * 8 + 8, :]) for fg, h in zip(ch, hv)]
                    pend.append((ch, hv))
                    if len(pend) > fskew:
                        second(*pend.pop(0))
                    yield len(hv) * 20 / 4 * fcost
                for p in pend:
                    second(*p)
                st["v"] = acc
            _interleave(vpu(), mxu())
            return residual(x + b2s[...] + jnp.concatenate(st["m"], axis=1), st["v"])

        def attn_dual(x, slot, never):
            y, r = center(x)
            yc = cols(y)
            scale = r * (DH ** -0.5 * LOG2E)
            link, hist, mhist = [None], [], []
            accm, accv, P = [None] * NC, [None] * NC, {}

            def lk(v):
                if not mchain or len(hist) < mchain:
                    return v.astype(BF16)
                c = cols(v)
                c[0] = jnp.where(never, hist[-mchain], c[0])
                return (jnp.concatenate(c, axis=1) if len(c) > 1 else c[0]).astype(BF16)

            def vk(v):
                if not vchain or len(mhist) < vchain:
                    return v
                return jnp.where(never, mhist[-vchain], v)

            def after(v):
                return v if link[0] is None else jnp.where(never, link[0], v)

            def mxu():
                for g in MG:
                    q = None
                    for j in range(G):
                        qj = mm(lk(y), bf(wqm[g * G + j]))
                        q = qj if q is None else jnp.where(row == j, qj, q)
                        mhist.append(qj)
                        yield 40 * mcost
                    s = None
                    for j in range(G):
                        sj = cols(mm(lk(q), bf(ktm[g * G + j])))
                        s = sj if s is None else [jnp.where(row == j, a, b) for a, b in zip(sj, s)]
                        mhist.append(sj[-1])
                        yield 64 * mcost
                    P[g] = softmax(s, scale)
                lhs = {}
                for g in MG:
                    p, inv = P[g]
                    pc = jnp.concatenate(p, axis=1)
                    o = []
                    for j in range(G):
                        o.append(mm(lk(pc), ldv(slot, g * G + j)))
                        mhist.append(o[-1])
                        yield 64 * mcost
                    lhs[g] = jnp.concatenate([jnp.where(row == j, o[j] * inv, 0.0) for j in range(G)], axis=1)
                for g in MG:
                    for c in range(NC):
                        a = mm(lk(lhs[g]), bf(wom[c, g * G * DH // 2:(g + 1) * G * DH // 2, :]))
                        accm[c] = a if accm[c] is None else accm[c] + a
                        mhist.append(a)
                        yield 64 * mcost

            def vpu():
                for i, g in enumerate(VG):
                    s = [None] * NKT
                    yg = [after(v) for v in yc]
                    for d in range(DH):
                        rs = slice(d * ST, d * ST + 8)
                        if d % dchunk == 0:
                            yd = [vk(yg[0])] + yg[1:]
                        qv = lanesum(_tree(add, [wqf[i, c, rs, :] * yd[c] for c in range(NC)]))
                        for t in range(NKT):
                            pr = ktf[i, t, rs, :] * qv
                            s[t] = pr if s[t] is None else s[t] + pr
                        if d == chain - 1:
                            link[0] = s[0]
                        if d % dchunk == dchunk - 1:
                            hist.append(s[-1])
                            yield dchunk * 25 / 4 * vcost
                    P[g] = softmax(s, scale)
                    yield 20
                for i, g in enumerate(VG):
                    p, inv = P[g]
                    inv = after(inv)
                    p = [t * inv for t in p]
                    for d in range(DH):
                        rs = slice(d * ST, d * ST + 8)
                        if d % dchunk == 0:
                            pd = [vk(p[0])] + p[1:]
                        ov = lanesum(_tree(add, [vtf[i, t, rs, :] * pd[t] for t in range(NKT)]))
                        for c in range(NC):
                            pr = wof[i, c, rs, :] * ov
                            accv[c] = pr if accv[c] is None else accv[c] + pr
                        if d == chain - 1:
                            link[0] = accv[0]
                        if d % dchunk == dchunk - 1:
                            hist.append(accv[-1])
                            yield dchunk * 25 / 4 * vcost
            _interleave(vpu(), mxu())
            return residual(x, [a + b for a, b in zip(accm, accv)])

        def rows_of(src, dst):
            n = src.shape[0]
            return _spread([(src.at[pl.ds(r, wrows), :], dst.at[pl.ds(r, wrows), :]) for r in range(0, n, wrows)], 8)
        small = [pltpu.make_async_copy(s, d, sems.at[S_SM]) for s, d in ((x_hbm, xb), (b1_hbm, b1v), (b2_hbm, b2v))]
        lq = _spread([(wq_hbm.at[pl.ds(r, 8), pl.ds(c, 1024)], wq.at[pl.ds(r, 8), pl.ds(c, 1024)])
                      for r in range(0, D, 8) for c in range(0, H * DH, 1024)], 8)
        for i, (s, d) in enumerate(lq):
            start(s, d, S_WQ)
            if i == 15:
                for c in small:
                    c.start()
        for s, d in rows_of(w1t_hbm, w1t):
            start(s, d, S_W1)
        for s, d in rows_of(wo_hbm, wo):
            start(s, d, S_WO)
        for s, d in rows_of(w2_hbm, w2):
            start(s, d, S_WO)
        for c in small:
            c.wait()
        x0 = xb[...].astype(F32)
        for i in range(B):
            xs[i] = jnp.broadcast_to(x0[i:i + 1, :], (8, D))
        b1s[...] = jnp.zeros((8, NF * 128), F32)
        b1s[:, 0:F] = jnp.broadcast_to(b1v[...].astype(F32).reshape(1, F), (8, F))
        b2s[...] = jnp.broadcast_to(b2v[...].astype(F32).reshape(1, D), (8, D))
        res[...] = jnp.zeros((8, D), F32)
        zero[...] = jnp.zeros((8, 128), F32)
        wait(wq, S_WQ)
        y0, r0 = center(x0)
        y0 = y0.astype(BF16)
        lanes = lambda i: pl.ds(pl.multiple_of(i * 128, 128), 128)

        @pl.loop(0, 8)
        def _(i):
            for j in range(16):
                kv_copy(0, 0, (i % 2) * 16 + j, i // 2, S_K)
            for j in range(4):
                h = i * 4 + j
                wt = wq[:, lanes(h)]
                wqm[h] = pltpu.bitcast(wt, U32)
                qa = mm(y0, wt) * r0
                for n in range(B):
                    q1[n, h] = jnp.broadcast_to(qa[n:n + 1, :], (8, DH))
        wait(w1t, S_W1)
        wait(wo, S_WO)
        wait(w2, S_WO)

        @pl.loop(0, 8)
        def _(i):
            for j in range(16):
                kv_copy(0, 0, (i % 2) * 16 + j, 4 + i // 2, S_K)
            for n, g in enumerate(VG if tail else ()):
                wt = bf(wqm[g * G + i]).T.astype(F32)
                for c in range(NC):
                    wqf[n, c, pl.ds(i, DH, stride=ST), :] = wt[:, c * 128:(c + 1) * 128]
            if compute:
                w1m[i] = pltpu.bitcast(w1t[lanes(i), :].T, U32)

                @pl.when(8 + i < F // 128)
                def _():
                    w1m[8 + i] = pltpu.bitcast(w1t[lanes(8 + i), :].T, U32)

            @pl.when(i < NC)
            def _():
                w2m[i, 0:F // 2, :] = pltpu.bitcast(w2[:, lanes(i)], U32)
                w2m[i, F // 2:NF * 64, :] = jnp.zeros((NF * 64 - F // 2, 128), U32)
                if tail:
                    w1f[i] = w1t[F - FV:F, lanes(i)].astype(F32)
                    w2f[i] = w2[F - FV:F, lanes(i)].astype(F32)
        if compute:
            w1m[NF - 1] = pltpu.bitcast(jnp.concatenate(
                [w1t[F // 128 * 128:F, :], jnp.zeros((NF * 128 - F, D), BF16)], axis=0).T, U32)

        @pl.loop(0, 8)
        def _(i):
            @pl.when(i < vpre)
            def _():
                for j in range(16):
                    kv_copy(1, 0, 16 + j, i, S_VHI)
            for c in range(NC):
                wom[c, pl.ds(pl.multiple_of(i * 256, 256), 256), :] = pltpu.bitcast(
                    wo[pl.ds(pl.multiple_of(i * 512, 512), 512), c * 128:(c + 1) * 128], U32)
                for n, g in enumerate(VG if tail else ()):
                    wof[n, c, pl.ds(i, DH, stride=ST), :] = wo[lanes(g * G + i), c * 128:(c + 1) * 128].astype(F32)
        for i in range(nfm, NF if tail else 0):
            b1c[(i - nfm) * 128:(i - nfm + 1) * 128, :] = jnp.broadcast_to(b1s[0:1, i * 128:(i + 1) * 128], (128, 128)).T

        c_att = DH ** -0.5 * LOG2E
        rowd = lax.broadcasted_iota(jnp.int32, (8, D), 0)

        def body(b, carry):
            slot = b % 2
            tick = Plan(kv_ticks(1, b, range(H // 2, H), S_VHI)[vpre:]
                        + kv_ticks(1, b, range(H // 2), S_VLO)
                        + kv_ticks(0, b + 1, range(H), S_K)
                        + kv_ticks(1, b + 1, range(H // 2, H), S_VHI)[:vpre])
            wait(kv.at[slot, 0], S_K)
            if not compute:
                tick(16 - vpre)
                wait(kv.at[slot, 1, pl.ds(H // 2, H // 2)], S_VHI)
                tick(pre_k)
                wait(kv.at[slot, 1, pl.ds(0, H // 2)], S_VLO)
                tick(len(tick.ticks) - tick.pos)
                return carry
            tick(8 - vpre)
            for g in range(NG):
                tick()
                p, inv = scores(slot, g, lambda j: q1[b, g * G + j].astype(BF16), c_att, tick)
                pscr[g] = jnp.concatenate(p, axis=1)
                lscr[g] = inv
            wait(kv.at[slot, 1, pl.ds(H // 2, H // 2)], S_VHI)
            acc = None
            for g in (2, 3):
                tick(2)
                acc = pv_wo(slot, range(g * G, (g + 1) * G), cols(pscr[g]), lscr[g], acc)
            tick(pre_k - 4)
            wait(kv.at[slot, 1, pl.ds(0, H // 2)], S_VLO)
            for g in (0, 1):
                tick()
                acc = pv_wo(slot, range(g * G, (g + 1) * G), cols(pscr[g]), lscr[g], acc)
            tick()
            x = mlp(residual(xs[b], acc), tick)
            tick()
            y, r = center(x)
            yb = y.astype(BF16)
            acc = None
            for g in range(NG):
                q = [mm(yb, bf(wqm[g * G + j])).astype(BF16) for j in range(G)]
                tick()
                p, inv = scores(slot, g, lambda j: q[j], r * c_att, tick)
                if g % 2:
                    tick()
                acc = pv_wo(slot, range(g * G, (g + 1) * G), p, inv, acc)
            x = mlp(residual(x, acc), tick)
            tick(len(tick.ticks) - tick.pos)
            res[...] = jnp.where(rowd == b, x, res[...])
            return carry

        lax.fori_loop(0, nb, body, 0)

        b = B - 1
        slot = b % 2
        pieces, h0 = [], 0
        for i, n in enumerate(last):
            pieces.append((range(h0, h0 + n), S_VLO + i))
            h0 += n
        assert h0 == H // 2
        ticks = (kv_ticks(1, b, range(H // 2, H), S_VHI)[vpre:]
                 + sum([kv_ticks(1, b, hs, sem, lastprio) for hs, sem in pieces], []))
        wait(kv.at[slot, 0], S_K)
        if not compute:
            for t in ticks:
                t()
            wait(kv.at[slot, 1, pl.ds(H // 2, H // 2)], S_VHI)
            for hs, sem in pieces:
                wait(kv.at[slot, 1, pl.ds(hs[0], len(hs))], sem)
            o_ref[...] = res[...].astype(BF16)
            return

        def ticks_at(i, lo, hi, n):
            for k in range(n):
                part = ticks[lo + (hi - lo) * k // n:lo + (hi - lo) * (k + 1) // n]
                if part:
                    @pl.when(i == k)
                    def _():
                        for t in part:
                            t()
        nt = len(ticks)
        cut = [0, (nt - 2) // 2, nt - 2, nt]
        for n, gs in enumerate((VG, MG)):
            @pl.loop(0, 2)
            def _(i):
                g = gs[0] + i
                ticks_at(i, cut[n], cut[n + 1], 2)
                p, inv = scores(slot, g, lambda j: q1[b, g * G + j].astype(BF16), c_att, lambda: None)
                pscr[g] = jnp.concatenate(p, axis=1)
                lscr[g] = inv
                for j in range(G if tail else 0):
                    kt = ldk(slot, g * G + j).T
                    if gs is MG:
                        ktm[g * G + j] = pltpu.bitcast(kt, U32)
                    else:
                        kt = kt.astype(F32)
                        for t in range(NKT):
                            ktf[i, t, pl.ds(j, DH, stride=ST), :] = kt[:, t * 128:(t + 1) * 128]
        wait(kv.at[slot, 1, pl.ds(H // 2, H // 2)], S_VHI)

        def upper(i, acc):
            g = VG[0] + i
            ticks_at(i, cut[2], cut[3], 2)
            pb = pscr[g].astype(BF16)
            parts = [jnp.where(row == j, mm(pb, ldv(slot, g * G + j)) * lscr[g], 0.0) for j in range(G)]
            lhs = jnp.concatenate(parts, axis=1).astype(BF16)
            rs = pl.ds(pl.multiple_of(g * (G * DH // 2), G * DH // 2), G * DH // 2)
            for j in range(G if tail else 0):
                vt = ldv(slot, g * G + j).T.astype(F32)
                for t in range(NKT):
                    vtf[i, t, pl.ds(j, DH, stride=ST), :] = vt[:, t * 128:(t + 1) * 128]
            return [acc[c] + mm(lhs, bf(wom[c, rs, :])) for c in range(NC)]
        acc = lax.fori_loop(0, 2, upper, [jnp.zeros((8, 128), F32)] * NC)
        for hs, sem in pieces:
            wait(kv.at[slot, 1, pl.ds(hs[0], len(hs))], sem if dma else 0)
            g = hs[0] // G
            acc = pv_wo(slot, hs, cols(pscr[g]), lscr[g], acc)
        x = residual(xs[b], acc)
        if tail == 2:
            x = x + jnp.tile(ktf[0, 0, 0:8, :] + vtf[0, 0, 0:8, :] + wqf[0, 0, 0:8, :] + wof[0, 0, 0:8, :] + w1f[0, 0:8, :] + w2f[0, 0:8, :]
                             + b1c[0:8, :] + pltpu.bitcast(ktm[0, 0:8, 0:128], F32), (1, NC))
        elif tail:
            never = zero[...] > 0.0
            x = mlp_dual(x, never)
            x = attn_dual(x, slot, never)
            x = mlp_dual(x, never)
        o_ref[...] = jnp.where(rowd == b, x, res[...]).astype(BF16)

    hbm = pl.BlockSpec(memory_space=pltpu.HBM)
    vm = pltpu.VMEM
    call = pl.pallas_call(
        kern,
        out_shape=jax.ShapeDtypeStruct((B, D), BF16),
        in_specs=[hbm] * 9,
        out_specs=pl.BlockSpec(memory_space=pltpu.VMEM),
        scratch_shapes=[
            vm((2, 2, H, W, DH), BF16),
            vm((D, H * DH), BF16), vm((H * DH, D), BF16), vm((F, D), BF16), vm((F, D), BF16),
            vm((B, D), BF16), vm((F,), BF16), vm((D,), BF16),
            vm((H, D // 2, DH), U32), vm((NC, H * DH // 2, 128), U32), vm((NF, D // 2, 128), U32), vm((NC, NF * 64, 128), U32),
            vm((2, NC, ST * DH, 128), F32), vm((2, NC, ST * DH, 128), F32),
            vm((NC, FV, 128), F32), vm((NC, FV, 128), F32), vm(((NF - nfm) * 128, 128), F32),
            vm((H // 2, DH // 2, W), U32), vm((2, NKT, ST * DH, 128), F32), vm((2, NKT, ST * DH, 128), F32),
            vm((B, 8, D), F32), vm((B, H, 8, DH), F32), vm((8, NF * 128), F32), vm((8, D), F32),
            vm((NG, 8, W), F32), vm((NG, 8, 128), F32), vm((B, D), F32), vm((8, 128), F32),
            pltpu.SemaphoreType.DMA((max(6, 2 + len(last)),)),
        ],
        compiler_params=pltpu.CompilerParams(
            vmem_limit_bytes=120 * 1024 * 1024, disable_bounds_checks=True, flags=flags),
    )

    return call


@jax.jit
def pallas_interleave_layers__sliding_block_cached__mixer_channel_mlp__decode_kernel(
    A_x, A_k_cache, A_v_cache, A_wq, A_wo, B_x, B_w1, B_b1, B_w2, B_b2):
    out = build()(A_x.reshape(B, D), A_k_cache, A_v_cache, A_wq, A_wo, B_w1.T, B_b1, B_w2, B_b2)
    return out.reshape(B, 1, D)
```

```python
import functools

import jax
import jax.numpy as jnp
from jax import lax
import jax.experimental.pallas as pl
import jax.experimental.pallas.tpu as pltpu

B, D, H, DH, SK, F = 8, 640, 32, 128, 4096, 1728
W = min(4096, max(256, SK // 4))
G = 8
NG = H // G
NC = D // 128
NK = W // 128
NF = -(-F // 128)
LAST = B - 1

F32, BF16, U32 = jnp.float32, jnp.bfloat16, jnp.uint32
SCORE_SCALE = DH ** -0.5 * 1.4426950408889634

KEYS_PER_COPY = 64
WEIGHT_ROWS_PER_COPY = 16
PRIORITIES = (0, 1, 1, 1)
STEP = 32
V_AHEAD = 4 * STEP
LAST_PIECES = (8, 5, 3)

MXU_GROUPS, VPU_GROUPS = (0, 1), (2, 3)
LOWER, UPPER = range(H // 2), range(H // 2, H)
CROSS = 7
PITCH = 12
PAD = 8
GUESS_MXU, GUESS_VPU = 1.07, 1.2 / 4

T_WQ = 0
T_WO = T_WQ + H * NC
T_W1 = T_WO + NC * H
T_W2 = T_W1 + NF * NC
T_V = T_W2 + NC * NF
T_END = T_V + len(LOWER) * NK

S_K, S_V_UPPER, S_V_LOWER = 0, 1, 2
S_SMALL, S_WQ, S_W1, S_WO = 2, 3, 4, 5


def _tree(op, xs):
    xs = list(xs)
    while len(xs) > 1:
        xs = [op(xs[i], xs[i + 1]) if i + 1 < len(xs) else xs[i] for i in range(0, len(xs), 2)]
    return xs[0]


def _spread(items, ways=8):
    per = -(-len(items) // ways)
    return [items[i] for r in range(per) for i in range(r, len(items), per)]


def _interleave(*streams):
    clock = [0.0] * len(streams)
    live = list(range(len(streams)))
    while live:
        for i in sorted(live, key=lambda i: clock[i]):
            cost = next(streams[i], False)
            if cost is False:
                live.remove(i)
                break
            if cost is not None:
                clock[i] += cost
                break
            clock[i] = max(clock[i], min((clock[j] for j in live if j != i), default=clock[i]))


def _mm(a, b):
    return jnp.dot(a, b, preferred_element_type=F32)


def _add(a, b):
    return a + b


def _cols(x):
    return [x[:, c:c + 128] for c in range(0, x.shape[1], 128)]


def _join(xs):
    return jnp.concatenate(list(xs), axis=1)


def _lane_sum(a):
    return jnp.broadcast_to(jnp.sum(a, axis=1, keepdims=True), (8, 128))


def _row_sum(a):
    return jnp.sum(a, axis=0, keepdims=True)


def _layernorm(x):
    d = x - jnp.mean(x, axis=-1, keepdims=True)
    var = jnp.mean(d * d, axis=-1, keepdims=True)
    return d, jnp.broadcast_to(lax.rsqrt(var + 1e-5), (8, 128))


def _gelu(x):
    c = 0.7978845608028654
    return 0.5 * x * (1.0 + jnp.tanh(x * (c + (c * 0.044715) * (x * x))))


def _softmax(s, scale):
    m = jnp.broadcast_to(jnp.max(_tree(jnp.maximum, s), axis=1, keepdims=True), (8, 128))
    p = [jnp.exp2((t - m) * scale) for t in s]
    return p, 1.0 / _lane_sum(_tree(_add, p))


def _kernel(x_hbm, k_hbm, v_hbm, wq_hbm, wo_hbm, w1t_hbm, b1_hbm, w2_hbm, b2_hbm,
            out_ref,
            kv, wq, wo, w1t, w2, x_in, b1_in, b2_in,
            mxu_tiles, k_mxu, wq_vpu, wo_vpu, w1_vpu, w2_vpu, k_vpu, v_vpu,
            x_rows, q_first, b1, b2, probs, inv_sum, result, zero, sems):
    row = lax.broadcasted_iota(jnp.int32, (8, 128), 0)
    out_row = lax.broadcasted_iota(jnp.int32, (8, D), 0)
    started = [0]

    def start(src, dst, sem):
        priority = PRIORITIES[started[0] % len(PRIORITIES)]
        started[0] += 1
        pltpu.make_async_copy(src, dst, sems.at[sem]).start(priority=priority)

    def wait(ref, sem):
        pltpu.make_async_copy(ref, ref, sems.at[sem]).wait()

    def window(which, heads, sem):
        return [(which, h, s, sem) for s in range(0, W, KEYS_PER_COPY) for h in heads]

    def start_kv(b, copies):
        for which, h, s, sem in copies:
            start((k_hbm, v_hbm)[which].at[b, h, pl.ds(SK - W + s, KEYS_PER_COPY), :],
                  kv.at[2 * (b % 2) + which, h, pl.ds(s, KEYS_PER_COPY), :], sem)

    def wait_kv(slot, which, heads, sem):
        wait(kv.at[2 * slot + which, pl.ds(heads[0], len(heads))], sem)

    def share(i, n, items, action, candidates=None):
        for k in candidates or range(n):
            part = items[len(items) * k // n:len(items) * (k + 1) // n]
            if part:
                pl.when(i == k)(functools.partial(action, part))

    def tiles(first, n):
        return pltpu.bitcast(jnp.concatenate([mxu_tiles[first + k, 0:64, :] for k in range(n)], axis=0), BF16)

    def put_tiles(first, w):
        words = pltpu.bitcast(w, U32)
        for k in range(w.shape[0] // 128):
            mxu_tiles[first + k, 0:64, :] = words[k * 64:(k + 1) * 64]

    def put_head(ref, group, j, w):
        w = w.astype(F32)
        for t, part in enumerate(_cols(w)):
            ref[group, t, pl.ds(j, DH, stride=PITCH), :] = part

    def lanes(i):
        return pl.ds(pl.multiple_of(i * 128, 128), 128)

    def rows_of(src, dst):
        n = WEIGHT_ROWS_PER_COPY
        return _spread([(src.at[pl.ds(r, n), :], dst.at[pl.ds(r, n), :]) for r in range(0, src.shape[0], n)])

    def start_all(sem, copies):
        for src, dst in copies:
            start(src, dst, sem)

    small = [pltpu.make_async_copy(src, dst, sems.at[S_SMALL])
             for src, dst in ((x_hbm, x_in), (b1_hbm, b1_in), (b2_hbm, b2_in))]
    wq_copies = _spread([(wq_hbm.at[pl.ds(r, 8), pl.ds(c, 1024)], wq.at[pl.ds(r, 8), pl.ds(c, 1024)])
                         for r in range(0, D, 8) for c in range(0, H * DH, 1024)])
    start_all(S_WQ, wq_copies[:16])
    for copy in small:
        copy.start()
    start_all(S_WQ, wq_copies[16:])
    start_all(S_W1, rows_of(w1t_hbm, w1t))
    for copy in small:
        copy.wait()
    x0 = x_in[...].astype(F32)
    for n in range(B):
        x_rows[n] = jnp.broadcast_to(x0[n:n + 1, :], (8, D))
    b1[...] = jnp.zeros((8, NF * 128), F32)
    b1[:, 0:F] = jnp.broadcast_to(b1_in[...].astype(F32).reshape(1, F), (8, F))
    b2[...] = jnp.broadcast_to(b2_in[...].astype(F32).reshape(1, D), (8, D))
    result[...] = jnp.zeros((B, D), F32)
    zero[...] = jnp.zeros((8, 128), F32)
    wait(wq, S_WQ)
    y0, r0 = _layernorm(x0)
    y0 = y0.astype(BF16)
    ahead = window(0, range(H), S_K) + window(1, UPPER, S_V_UPPER)[:V_AHEAD]

    @pl.loop(0, G)
    def _(j):
        share(j, G, rows_of(wo_hbm, wo), functools.partial(start_all, S_WO))
        for g in range(NG):
            h = g * G + j
            w = wq[:, lanes(h)]
            put_tiles(T_WQ + h * NC, w)
            q = _mm(y0, w) * r0
            for n in range(B):
                q_first[n, h] = jnp.broadcast_to(q[n:n + 1, :], (8, DH))
            if g in VPU_GROUPS:
                put_head(wq_vpu, g - VPU_GROUPS[0], j, w.T)

    wait(w1t, S_W1)

    @pl.loop(0, 7)
    def _(i):
        share(i, 4, rows_of(w2_hbm, w2), functools.partial(start_all, S_WO))
        share(i - 4, 3, ahead[:4 * STEP], functools.partial(start_kv, 0))
        put_tiles(T_W1 + i * NC, w1t[lanes(i), :].T)

        @pl.when(7 + i < F // 128)
        def _():
            put_tiles(T_W1 + (7 + i) * NC, w1t[lanes(7 + i), :].T)

        @pl.when(i < NC)
        def _():
            w1_vpu[i, 0:F - CROSS * 128, :] = w1t[CROSS * 128:F, lanes(i)].astype(F32)

    put_tiles(T_W1 + (NF - 1) * NC,
              jnp.concatenate([w1t[F // 128 * 128:F, :], jnp.zeros((NF * 128 - F, D), BF16)], axis=0).T)
    wait(wo, S_WO)
    wait(w2, S_WO)

    @pl.loop(0, G)
    def _(j):
        share(j, G, ahead[4 * STEP:], functools.partial(start_kv, 0))
        for c in range(NC):
            put_tiles(T_WO + c * H + 4 * j, wo[pl.ds(pl.multiple_of(j * 512, 512), 512), c * 128:(c + 1) * 128])
        for i, g in enumerate(VPU_GROUPS):
            put_head(wo_vpu, i, j, wo[lanes(g * G + j), :])

        @pl.when(j < NC)
        def _():
            put_tiles(T_W2 + j * NF,
                      jnp.concatenate([w2[:, lanes(j)], jnp.zeros((NF * 128 - F, 128), BF16)], axis=0))
            w2_vpu[j, 0:CROSS * 128, :] = w2[0:CROSS * 128, lanes(j)].astype(F32)

    def scores(slot, g, q, tick):
        s = None
        for j in range(G):
            sj = _cols(lax.dot_general(q(j), kv[2 * slot, g * G + j], (((1,), (1,)), ((), ())),
                                       preferred_element_type=F32))
            s = sj if s is None else [jnp.where(row == j, a, b) for a, b in zip(sj, s)]
            tick(128)
        return s

    def values(slot, heads, p, inv, acc, tick=lambda work: None, keep=False):
        p = _join(p).astype(BF16)
        o = []
        for h in heads:
            v = kv[2 * slot + 1, h]
            o.append(jnp.where(row == h % G, _mm(p, v) * inv, 0.0))
            if keep:
                put_tiles(T_V + h * NK, v)
            tick(64)
        o = _join(o).astype(BF16)
        out = []
        for c in range(NC):
            out.append(_mm(o, tiles(T_WO + c * H + heads[0], len(heads))))
            tick(8 * len(heads))
        return out if acc is None else [a + b for a, b in zip(acc, out)]

    def mlp(x, tick):
        y, r = _layernorm(x)
        y = y.astype(BF16)
        hidden = []
        for i in range(NF):
            hidden.append(_gelu(_mm(y, tiles(T_W1 + i * NC, NC)) * r + b1[:, i * 128:(i + 1) * 128]))
            tick(40)
        hidden = _join(hidden).astype(BF16)
        out = []
        for c in range(NC):
            out.append(_mm(hidden, tiles(T_W2 + c * NF, NF)))
            tick(8 * NF)
        return x + b2[...] + _join(out)

    @pl.loop(0, LAST)
    def _(b):
        slot = b % 2
        todo = [(b, c) for c in window(1, UPPER, S_V_UPPER)[V_AHEAD:] + window(1, LOWER, S_V_LOWER)]
        v_end = len(todo)
        todo += [(b + 1, c) for c in ahead]
        done = [0]

        def ticker(end, work):
            begin, seen = done[0], [0]

            def tick(n):
                seen[0] += n
                while done[0] < begin + (end - begin) * seen[0] // work:
                    start_kv(todo[done[0]][0], [todo[done[0]][1]])
                    done[0] += 1
            return tick

        group = lambda g: range(g * G, (g + 1) * G)
        wait_kv(slot, 0, range(H), S_K)
        tick = ticker(v_end - 2 * STEP, H * 128)
        for g in range(NG):
            p, inv = _softmax(scores(slot, g, lambda j: q_first[b, g * G + j].astype(BF16), tick), SCORE_SCALE)
            probs[g] = _join(p)
            inv_sum[g] = inv
        wait_kv(slot, 1, UPPER, S_V_UPPER)
        acc = None
        tick = ticker(v_end + 2 * STEP, len(UPPER) * 104)
        for g in VPU_GROUPS:
            acc = values(slot, group(g), _cols(probs[g]), inv_sum[g], acc, tick)
        wait_kv(slot, 1, LOWER, S_V_LOWER)
        tick = ticker(len(todo), len(LOWER) * 104 + 2 * 80 * NF + H * 272)
        for g in MXU_GROUPS:
            acc = values(slot, group(g), _cols(probs[g]), inv_sum[g], acc, tick)
        x = mlp(x_rows[b] + _row_sum(_join(acc)), tick)

        y, r = _layernorm(x)
        y = y.astype(BF16)
        acc = None
        for g in range(NG):
            q = []
            for h in group(g):
                q.append(_mm(y, tiles(T_WQ + h * NC, NC)).astype(BF16))
                tick(40)
            p, inv = _softmax(scores(slot, g, lambda j: q[j], tick), r * SCORE_SCALE)
            acc = values(slot, group(g), p, inv, acc, tick)
        x = mlp(x + _row_sum(_join(acc)), tick)
        assert done[0] == len(todo)
        result[...] = jnp.where(out_row == b, x, result[...])

    def shared_mlp(x):
        y, r = _layernorm(x)
        y_mxu, y_vpu = y.astype(BF16), _cols(y)
        hidden, turned, out = {}, {}, {}

        def activate(i, h):
            hidden[i] = _gelu(h * r + b1[:, i * 128:(i + 1) * 128])

        def mxu():
            for i in range(CROSS):
                activate(i, _mm(y_mxu, tiles(T_W1 + i * NC, NC)))
                yield 40 * GUESS_MXU
            acc = [None] * NC
            for i in range(CROSS, NF):
                while i not in hidden:
                    yield None
                n = min(128, F - i * 128)
                h = hidden[i].astype(BF16)[:, 0:n]
                for c in range(NC):
                    a = _mm(h, pltpu.bitcast(mxu_tiles[T_W2 + c * NF + i, 0:n // 2, :], BF16))
                    acc[c] = a if acc[c] is None else acc[c] + a
                yield n / 128 * 40 * GUESS_MXU
            out["mxu"] = acc

        def turn(i):
            if i < CROSS:
                while i not in hidden:
                    yield None
                turned[i] = jnp.concatenate([hidden[i]] * 16, axis=0).astype(BF16).T

        def vpu():
            for i in range(CROSS, NF):
                n = min(128, F - i * 128)
                first = (i - CROSS) * 128
                parts = [_tree(_add, [w1_vpu[c, f:f + 8, :] * y_vpu[c] for c in range(NC)])
                         for f in range(first, first + n, 8)]
                parts += [jnp.zeros((8, 128), F32)] * (16 - len(parts))
                parts = jnp.concatenate(parts, axis=0).T
                h = _row_sum(_tree(_add, [parts[k:k + 8] for k in range(0, 128, 8)]))
                activate(i, jnp.broadcast_to(h, (8, 128)))
                yield n / 128 * 43
            yield from turn(0)
            acc = [None] * NC
            for i in range(CROSS):
                yield from turn(i + 1)
                h = turned[i].astype(F32)
                for k in range(0, 128, 16):
                    f = i * 128 + k
                    for c in range(NC):
                        a = w2_vpu[c, f:f + 8, :] * h[k:k + 8] + w2_vpu[c, f + 8:f + 16, :] * h[k + 8:k + 16]
                        acc[c] = a if acc[c] is None else acc[c] + a
                yield 40
            out["vpu"] = acc

        _interleave(vpu(), mxu())
        return x + b2[...] + _join(out["mxu"]) + _row_sum(_join(out["vpu"]))

    def shared_attention(x):
        y, r = _layernorm(x)
        scale = r * SCORE_SCALE
        p_of, acc_mxu, acc_vpu = {}, [None] * NC, [None] * NC
        never = zero[...] > 0.0
        mxu_trail, vpu_trail, previous_task = [], [], []

        def not_before(trail, lag, value):
            return value if len(trail) < lag else jnp.where(never, trail[-lag], value)

        def lhs(value):
            head, *rest = _cols(value)
            return _join([not_before(vpu_trail, 24, head)] + rest).astype(BF16)

        def paced(values):
            return [not_before(mxu_trail, 6, values[0])] + values[1:]

        def mxu():
            q_of, o_of = {}, {}
            for g in MXU_GROUPS:
                q = None
                for j in range(G):
                    qj = _mm(lhs(y), tiles(T_WQ + (g * G + j) * NC, NC))
                    q = qj if q is None else jnp.where(row == j, qj, q)
                    mxu_trail.append(qj)
                    yield 40 * GUESS_MXU
                q_of[g] = q
            for g in MXU_GROUPS:
                s = None
                for j in range(G):
                    sj = _cols(_mm(lhs(q_of[g]), pltpu.bitcast(k_mxu[g * G + j], BF16)))
                    s = sj if s is None else [jnp.where(row == j, a, b) for a, b in zip(sj, s)]
                    mxu_trail.append(sj[-1])
                    yield 64 * GUESS_MXU
                p_of[g] = _softmax(s, scale)
            for g in MXU_GROUPS:
                p, inv = p_of[g]
                o = []
                for j in range(G):
                    o.append(_mm(lhs(_join(p)), tiles(T_V + (g * G + j) * NK, NK)))
                    mxu_trail.append(o[-1])
                    yield 64 * GUESS_MXU
                o_of[g] = _join(jnp.where(row == j, o[j] * inv, 0.0) for j in range(G))
            for g in MXU_GROUPS:
                for c in range(NC):
                    a = _mm(lhs(o_of[g]), tiles(T_WO + c * H + g * G, G))
                    acc_mxu[c] = a if acc_mxu[c] is None else acc_mxu[c] + a
                    mxu_trail.append(a)
                    yield 64 * GUESS_MXU

        def contract(first, factors, second, acc):
            for d in range(DH):
                rows = slice(d * PITCH, d * PITCH + 8)
                terms = [first(t, rows) * f for t, f in enumerate(paced(factors))]
                value = _lane_sum(functools.reduce(_add, terms) if len(terms) == NC else _tree(_add, terms))
                for t in range(len(acc)):
                    a = second(t, rows) * value
                    acc[t] = a if acc[t] is None else acc[t] + a
                if d == 87:
                    previous_task.append(acc[0])
                vpu_trail.append(acc[-1])
                yield 25 * GUESS_VPU

        def vpu():
            for i, g in enumerate(VPU_GROUPS):
                s = [None] * NK
                yield from contract(lambda c, rows: wq_vpu[i, c, rows, :],
                                    [not_before(previous_task, 1, v) for v in _cols(y)],
                                    lambda t, rows: k_vpu[i, t, rows, :], s)
                p_of[g] = _softmax(s, scale)
                yield 20
            for i, g in enumerate(VPU_GROUPS):
                p, inv = p_of[g]
                inv = not_before(previous_task, 1, inv)
                yield from contract(lambda t, rows: v_vpu[i, t, rows, :], [t * inv for t in p],
                                    lambda c, rows: wo_vpu[i, c, rows, :], acc_vpu)

        _interleave(vpu(), mxu())
        return x + _row_sum(_join(a + b for a, b in zip(acc_mxu, acc_vpu)))

    slot = LAST % 2
    pieces, first_head = [], 0
    for i, n in enumerate(LAST_PIECES):
        pieces.append((range(first_head, first_head + n), S_V_LOWER + i))
        first_head += n
    copies = window(1, UPPER, S_V_UPPER)[V_AHEAD:]
    for heads, sem in pieces:
        copies += window(1, heads, sem)
    start_last = functools.partial(start_kv, LAST)
    wait_kv(slot, 0, range(H), S_K)

    @pl.loop(0, 2)
    def _(i):
        for n, g in enumerate((VPU_GROUPS[0] + i, MXU_GROUPS[0] + i)):
            s = None
            for j in range(G):
                step = G * n + j
                share(2 * G * i + step, 4 * G, copies[:-4 * STEP], start_last, (step, 2 * G + step))
                k = kv[2 * slot, g * G + j].T
                sj = _cols(_mm(q_first[LAST, g * G + j].astype(BF16), k))
                s = sj if s is None else [jnp.where(row == j, a, b) for a, b in zip(sj, s)]
                if n:
                    k_mxu[g * G + j] = pltpu.bitcast(k, U32)
                else:
                    put_head(k_vpu, i, j, k)
            p, inv = _softmax(s, SCORE_SCALE)
            probs[g] = _join(p)
            inv_sum[g] = inv

    def upper_values(i, acc):
        g = VPU_GROUPS[0] + i
        p = probs[g].astype(BF16)
        o = []
        for j in range(G):
            share(G * i + j, 2 * G, copies[-4 * STEP:], start_last, (j, G + j))
            v = kv[2 * slot + 1, g * G + j]
            o.append(jnp.where(row == j, _mm(p, v) * inv_sum[g], 0.0))
            put_head(v_vpu, i, j, v.T)
        o = _join(o).astype(BF16)
        return [acc[c] + _mm(o, tiles(T_WO + c * H + g * G, G)) for c in range(NC)]

    wait_kv(slot, 1, UPPER, S_V_UPPER)
    acc = lax.fori_loop(0, 2, upper_values, [jnp.zeros((8, 128), F32)] * NC)
    for heads, sem in pieces:
        wait_kv(slot, 1, heads, sem)
        g = heads[0] // G
        acc = values(slot, heads, _cols(probs[g]), inv_sum[g], acc, keep=True)
    x = x_rows[LAST] + _row_sum(_join(acc))
    x = shared_mlp(shared_attention(shared_mlp(x)))
    out_ref[...] = jnp.where(out_row == LAST, x, result[...]).astype(out_ref.dtype)


@jax.jit
def pallas_interleave_layers__sliding_block_cached__mixer_channel_mlp__decode_kernel(
    A_x: jax.Array,
    A_k_cache: jax.Array,
    A_v_cache: jax.Array,
    A_wq: jax.Array,
    A_wo: jax.Array,
    B_x: jax.Array,
    B_w1: jax.Array,
    B_b1: jax.Array,
    B_w2: jax.Array,
    B_b2: jax.Array,
):
    vmem = pltpu.VMEM
    features = PITCH * DH + PAD
    out = pl.pallas_call(
        _kernel,
        out_shape=jax.ShapeDtypeStruct((B, D), A_x.dtype),
        in_specs=[pl.BlockSpec(memory_space=pltpu.HBM)] * 9,
        out_specs=pl.BlockSpec(memory_space=pltpu.VMEM),
        scratch_shapes=[
            vmem((4, H, W, DH), BF16),
            vmem((D, H * DH), BF16), vmem((H * DH, D), BF16), vmem((F, D), BF16), vmem((F, D), BF16),
            vmem((B, D), BF16), vmem((F,), BF16), vmem((D,), BF16),
            vmem((T_END, 64 + PAD, 128), U32),
            vmem((len(LOWER), DH // 2, W), U32),
            vmem((2, NC, features, 128), F32), vmem((2, NC, features, 128), F32),
            vmem((NC, F - CROSS * 128 + PAD, 128), F32), vmem((NC, CROSS * 128 + PAD, 128), F32),
            vmem((2, NK, features, 128), F32), vmem((2, NK, features, 128), F32),
            vmem((B, 8, D), F32), vmem((B, H, 8, DH), F32), vmem((8, NF * 128), F32), vmem((8, D), F32),
            vmem((NG, 8, W), F32), vmem((NG, 8, 128), F32), vmem((B, D), F32), vmem((8, 128), F32),
            pltpu.SemaphoreType.DMA((6,)),
        ],
        compiler_params=pltpu.CompilerParams(
            vmem_limit_bytes=124 * 1024 * 1024, disable_bounds_checks=True),
    )(A_x.reshape(B, D), A_k_cache, A_v_cache, A_wq, A_wo, B_w1.T, B_b1, B_w2, B_b2)
    return out.reshape(B, 1, D)
```

```python
import functools

import jax
import jax.numpy as jnp
from jax import lax
import jax.experimental.pallas as pl
import jax.experimental.pallas.tpu as pltpu

B, D, H, DH, SK, F = 8, 640, 32, 128, 4096, 1728
W = min(4096, max(256, SK // 4))
G = 8
NG = H // G
NC = D // 128
NK = W // 128
NF = -(-F // 128)
LAST = B - 1

F32, BF16, U32 = jnp.float32, jnp.bfloat16, jnp.uint32
SCORE_SCALE = DH ** -0.5 * 1.4426950408889634

KEYS_PER_COPY = 64
WEIGHT_ROWS_PER_COPY = 16
PRIORITIES = (0, 1, 1, 1)
STEP = 32
V_AHEAD = 4 * STEP
LAST_PIECES = (8, 5, 3)

MXU_GROUPS, VPU_GROUPS = (0, 1), (2, 3)
LOWER, UPPER = range(H // 2), range(H // 2, H)
CROSS = 6
PITCH = 12
PAD = 8
GUESS_MXU, GUESS_VPU = 1.07, 1.2 / 4

T_WQ = 0
T_WO = T_WQ + H * NC
T_W1 = T_WO + NC * H
T_W2 = T_W1 + NF * NC
T_V = T_W2 + NC * NF
T_END = T_V + len(LOWER) * NK

S_K, S_V_UPPER, S_V_LOWER = 0, 1, 2
S_SMALL, S_WQ, S_W1, S_WO = 2, 3, 4, 5


def _tree(op, xs):
    xs = list(xs)
    while len(xs) > 1:
        xs = [op(xs[i], xs[i + 1]) if i + 1 < len(xs) else xs[i] for i in range(0, len(xs), 2)]
    return xs[0]


def _spread(items, ways=8):
    per = -(-len(items) // ways)
    return [items[i] for r in range(per) for i in range(r, len(items), per)]


def _interleave(*streams):
    clock = [0.0] * len(streams)
    live = list(range(len(streams)))
    while live:
        for i in sorted(live, key=lambda i: clock[i]):
            cost = next(streams[i], False)
            if cost is False:
                live.remove(i)
                break
            if cost is not None:
                clock[i] += cost
                break
            clock[i] = max(clock[i], min((clock[j] for j in live if j != i), default=clock[i]))


def _mm(a, b):
    return jnp.dot(a, b, preferred_element_type=F32)


def _add(a, b):
    return a + b


def _sum(xs):
    return functools.reduce(_add, xs)


def _cols(x):
    return [x[:, c:c + 128] for c in range(0, x.shape[1], 128)]


def _join(xs):
    return jnp.concatenate(list(xs), axis=1)


def _lane_sum(a):
    return jnp.broadcast_to(jnp.sum(a, axis=1, keepdims=True), (8, 128))


def _row_sum(a):
    return jnp.sum(a, axis=0, keepdims=True)


def _layernorm(x):
    d = x - jnp.mean(x, axis=-1, keepdims=True)
    var = jnp.mean(d * d, axis=-1, keepdims=True)
    return d, jnp.broadcast_to(lax.rsqrt(var + 1e-5), (8, 128))


def _gelu(x):
    c = 0.7978845608028654
    return 0.5 * x * (1.0 + jnp.tanh(x * (c + (c * 0.044715) * (x * x))))


def _softmax(s, scale):
    m = jnp.broadcast_to(jnp.max(_tree(jnp.maximum, s), axis=1, keepdims=True), (8, 128))
    p = [jnp.exp2((t - m) * scale) for t in s]
    return p, 1.0 / _lane_sum(_tree(_add, p))


def _kernel(x_hbm, k_hbm, v_hbm, wq_hbm, wo_hbm, w1t_hbm, b1_hbm, w2_hbm, b2_hbm,
            out_ref,
            kv, wq, wo, w1t, w2, x_in, b1_in, b2_in,
            mxu_tiles, k_mxu, wq_vpu, wo_vpu, w1_vpu, w2_vpu, k_vpu, v_vpu,
            x_rows, q_first, b1, b2, probs, inv_sum, result, zero, sems):
    row = lax.broadcasted_iota(jnp.int32, (8, 128), 0)
    out_row = lax.broadcasted_iota(jnp.int32, (8, D), 0)
    started = [0]

    def start(src, dst, sem):
        priority = PRIORITIES[started[0] % len(PRIORITIES)]
        started[0] += 1
        pltpu.make_async_copy(src, dst, sems.at[sem]).start(priority=priority)

    def wait(ref, sem):
        pltpu.make_async_copy(ref, ref, sems.at[sem]).wait()

    def window(which, heads, sem):
        return [(which, h, s, sem) for s in range(0, W, KEYS_PER_COPY) for h in heads]

    def start_kv(b, copies):
        for which, h, s, sem in copies:
            if not isinstance(s, int):
                s = pl.multiple_of(s, KEYS_PER_COPY)
            start((k_hbm, v_hbm)[which].at[b, h, pl.ds(SK - W + s, KEYS_PER_COPY), :],
                  kv.at[2 * (b % 2) + which, h, pl.ds(s, KEYS_PER_COPY), :], sem)

    def wait_kv(slot, which, heads, sem):
        wait(kv.at[2 * slot + which, pl.ds(heads[0], len(heads))], sem)

    def share(i, n, items, action, candidates=None):
        for k in candidates or range(n):
            part = items[len(items) * k // n:len(items) * (k + 1) // n]
            if part:
                pl.when(i == k)(functools.partial(action, part))

    def tiles(first, n):
        return pltpu.bitcast(jnp.concatenate([mxu_tiles[first + k, 0:64, :] for k in range(n)], axis=0), BF16)

    def put_tiles(first, w):
        words = pltpu.bitcast(w, U32)
        for k in range(w.shape[0] // 128):
            mxu_tiles[first + k, 0:64, :] = words[k * 64:(k + 1) * 64]

    def put_head(ref, group, j, w):
        w = w.astype(F32)
        for t, part in enumerate(_cols(w)):
            ref[group, t, pl.ds(j, DH, stride=PITCH), :] = part

    def lanes(i):
        return pl.ds(pl.multiple_of(i * 128, 128), 128)

    def rows_of(src, dst):
        n = WEIGHT_ROWS_PER_COPY
        return _spread([(src.at[pl.ds(r, n), :], dst.at[pl.ds(r, n), :]) for r in range(0, src.shape[0], n)])

    def start_all(sem, copies):
        for src, dst in copies:
            start(src, dst, sem)

    small = [pltpu.make_async_copy(src, dst, sems.at[S_SMALL])
             for src, dst in ((x_hbm, x_in), (b1_hbm, b1_in), (b2_hbm, b2_in))]
    wq_copies = _spread([(wq_hbm.at[pl.ds(r, 8), pl.ds(c, 1024)], wq.at[pl.ds(r, 8), pl.ds(c, 1024)])
                         for r in range(0, D, 8) for c in range(0, H * DH, 1024)])
    start_all(S_WQ, wq_copies[:16])
    for copy in small:
        copy.start()
    start_all(S_WQ, wq_copies[16:])
    start_all(S_W1, rows_of(w1t_hbm, w1t))
    for copy in small:
        copy.wait()
    x0 = x_in[...].astype(F32)
    for n in range(B):
        x_rows[n] = jnp.broadcast_to(x0[n:n + 1, :], (8, D))
    b1[...] = jnp.zeros((8, NF * 128), F32)
    b1[:, 0:F] = jnp.broadcast_to(b1_in[...].astype(F32).reshape(1, F), (8, F))
    b2[...] = jnp.broadcast_to(b2_in[...].astype(F32).reshape(1, D), (8, D))
    result[...] = jnp.zeros((B, D), F32)
    zero[...] = jnp.zeros((8, 128), F32)
    wait(wq, S_WQ)
    y0, r0 = _layernorm(x0)
    y0 = y0.astype(BF16)
    ahead = window(0, range(H), S_K) + window(1, UPPER, S_V_UPPER)[:V_AHEAD]

    @pl.loop(0, G)
    def _(j):
        for m in range(32):
            r = pl.multiple_of((m % 8 * 32 + m // 8 + 4 * j) * WEIGHT_ROWS_PER_COPY, WEIGHT_ROWS_PER_COPY)
            start(wo_hbm.at[pl.ds(r, WEIGHT_ROWS_PER_COPY), :], wo.at[pl.ds(r, WEIGHT_ROWS_PER_COPY), :], S_WO)
        for g in range(NG):
            h = g * G + j
            w = wq[:, lanes(h)]
            put_tiles(T_WQ + h * NC, w)
            q = _mm(y0, w) * r0
            for n in range(B):
                q_first[n, h] = jnp.broadcast_to(q[n:n + 1, :], (8, DH))
            if g in VPU_GROUPS:
                put_head(wq_vpu, g - VPU_GROUPS[0], j, w.T)

    wait(w1t, S_W1)

    @pl.loop(0, 7)
    def _(i):
        share(i, 4, rows_of(w2_hbm, w2), functools.partial(start_all, S_WO))
        share(i - 4, 3, ahead[:4 * STEP], functools.partial(start_kv, 0))
        put_tiles(T_W1 + i * NC, w1t[lanes(i), :].T)

        @pl.when(7 + i < F // 128)
        def _():
            put_tiles(T_W1 + (7 + i) * NC, w1t[lanes(7 + i), :].T)

        @pl.when(i < NC)
        def _():
            w1_vpu[i, 0:F - CROSS * 128, :] = w1t[CROSS * 128:F, lanes(i)].astype(F32)

    put_tiles(T_W1 + (NF - 1) * NC,
              jnp.concatenate([w1t[F // 128 * 128:F, :], jnp.zeros((NF * 128 - F, D), BF16)], axis=0).T)
    wait(wo, S_WO)
    wait(w2, S_WO)

    @pl.loop(0, G)
    def _(j):
        pl.when(j < 6)(lambda: start_kv(0, [(0, h, (4 + 2 * j + m) * KEYS_PER_COPY, S_K)
                                            for m in range(2) for h in range(H)]))
        pl.when(j >= 6)(lambda: start_kv(0, [(1, h, (4 * (j - 6) + m) * KEYS_PER_COPY, S_V_UPPER)
                                             for m in range(4) for h in UPPER]))
        for c in range(NC):
            put_tiles(T_WO + c * H + 4 * j, wo[pl.ds(pl.multiple_of(j * 512, 512), 512), c * 128:(c + 1) * 128])
        for i, g in enumerate(VPU_GROUPS):
            put_head(wo_vpu, i, j, wo[lanes(g * G + j), :])

        @pl.when(j < NC)
        def _():
            put_tiles(T_W2 + j * NF,
                      jnp.concatenate([w2[:, lanes(j)], jnp.zeros((NF * 128 - F, 128), BF16)], axis=0))
            w2_vpu[j, 0:CROSS * 128, :] = w2[0:CROSS * 128, lanes(j)].astype(F32)

    def scores(slot, g, q, tick):
        s = None
        for j in range(G):
            sj = _cols(lax.dot_general(q(j), kv[2 * slot, g * G + j], (((1,), (1,)), ((), ())),
                                       preferred_element_type=F32))
            s = sj if s is None else [jnp.where(row == j, a, b) for a, b in zip(sj, s)]
            tick(128)
        return s

    def values(slot, heads, p, inv, acc, tick=lambda work: None, keep=False):
        p = _join(p).astype(BF16)
        o = []
        for h in heads:
            v = kv[2 * slot + 1, h]
            o.append(jnp.where(row == h % G, _mm(p, v) * inv, 0.0))
            if keep:
                put_tiles(T_V + h * NK, v)
            tick(64)
        o = _join(o).astype(BF16)
        out = []
        for c in range(NC):
            out.append(_mm(o, tiles(T_WO + c * H + heads[0], len(heads))))
            tick(8 * len(heads))
        return out if acc is None else [a + b for a, b in zip(acc, out)]

    def mlp(x, tick):
        y, r = _layernorm(x)
        y = y.astype(BF16)
        hidden = []
        for i in range(NF):
            hidden.append(_gelu(_mm(y, tiles(T_W1 + i * NC, NC)) * r + b1[:, i * 128:(i + 1) * 128]))
            tick(40)
        hidden = _join(hidden).astype(BF16)
        out = []
        for c in range(NC):
            out.append(_mm(hidden, tiles(T_W2 + c * NF, NF)))
            tick(8 * NF)
        return x + b2[...] + _join(out)

    @pl.loop(0, LAST)
    def _(b):
        slot = b % 2
        upper, lower = window(1, UPPER, S_V_UPPER)[V_AHEAD:], window(1, LOWER, S_V_LOWER)
        todo = []
        for i in range(0, len(lower), H // 2):
            todo += [(b, c) for c in lower[i:i + H // 2] + upper[i:i + H // 2]]
        v_end = len(todo)
        todo += [(b + 1, c) for c in ahead]
        done = [0]

        def ticker(end, work):
            begin, seen = done[0], [0]

            def tick(n):
                seen[0] += n
                while done[0] < begin + (end - begin) * seen[0] // work:
                    start_kv(todo[done[0]][0], [todo[done[0]][1]])
                    done[0] += 1
            return tick

        group = lambda g: range(g * G, (g + 1) * G)
        wait_kv(slot, 0, range(H), S_K)
        tick = ticker(v_end - 2 * STEP, H * 128)
        for g in range(NG):
            p, inv = _softmax(scores(slot, g, lambda j: q_first[b, g * G + j].astype(BF16), tick), SCORE_SCALE)
            probs[g] = _join(p)
            inv_sum[g] = inv
        wait_kv(slot, 1, UPPER, S_V_UPPER)
        acc = None
        tick = ticker(v_end + 2 * STEP, len(UPPER) * 104)
        for g in VPU_GROUPS:
            acc = values(slot, group(g), _cols(probs[g]), inv_sum[g], acc, tick)
        wait_kv(slot, 1, LOWER, S_V_LOWER)
        tick = ticker(len(todo), len(LOWER) * 104 + 2 * 80 * NF + H * 272)
        for g in MXU_GROUPS:
            acc = values(slot, group(g), _cols(probs[g]), inv_sum[g], acc, tick)
        x = mlp(x_rows[b] + _row_sum(_join(acc)), tick)

        y, r = _layernorm(x)
        y = y.astype(BF16)
        acc = None
        for g in range(NG):
            q = []
            for h in group(g):
                q.append(_mm(y, tiles(T_WQ + h * NC, NC)).astype(BF16))
                tick(40)
            p, inv = _softmax(scores(slot, g, lambda j: q[j], tick), r * SCORE_SCALE)
            acc = values(slot, group(g), p, inv, acc, tick)
        x = mlp(x + _row_sum(_join(acc)), tick)
        assert done[0] == len(todo)
        result[...] = jnp.where(out_row == b, x, result[...])

    def shared_mlp(x):
        y, r = _layernorm(x)
        y_mxu, y_vpu = y.astype(BF16), _cols(y)
        hidden, turned, out = {}, {}, {}
        crossed = [NF - 1] + list(range(CROSS, NF - 1))
        width = lambda i: min(128, F - i * 128)

        def activate(i, h):
            n = width(i)
            hidden[i] = _gelu(h * r[:, 0:n] + b1[:, i * 128:i * 128 + n])

        def mxu():
            for i in range(CROSS):
                activate(i, _mm(y_mxu, tiles(T_W1 + i * NC, NC)))
                yield 40 * GUESS_MXU
            acc = [None] * NC
            for i in crossed:
                while i not in hidden:
                    yield None
                h = hidden[i].astype(BF16)
                for c in range(NC):
                    a = _mm(h, pltpu.bitcast(mxu_tiles[T_W2 + c * NF + i, 0:width(i) // 2, :], BF16))
                    acc[c] = a if acc[c] is None else acc[c] + a
                yield width(i) / 128 * 40 * GUESS_MXU
            out["mxu"] = acc

        def turn(i):
            if i < CROSS:
                while i not in hidden:
                    yield None
                turned[i] = jnp.concatenate([hidden[i]] * 16, axis=0).astype(BF16).T

        def vpu():
            for i in crossed:
                first = (i - CROSS) * 128
                parts = [_sum([w1_vpu[c, f:f + 8, :] * y_vpu[c] for c in range(NC)])
                         for f in range(first, first + width(i), 8)]
                parts = jnp.concatenate(parts, axis=0).T
                h = _row_sum(_sum([parts[k:k + 8] for k in range(0, 128, 8)]))
                activate(i, jnp.broadcast_to(h, (8, width(i))))
                yield width(i) / 128 * 43
            yield from turn(0)
            yield from turn(1)
            acc = [None] * NC
            for i in range(CROSS):
                yield from turn(i + 2)
                h = turned[i].astype(F32)
                for k in range(0, 128, 16):
                    f = i * 128 + k
                    for c in range(NC):
                        a = w2_vpu[c, f:f + 8, :] * h[k:k + 8] + w2_vpu[c, f + 8:f + 16, :] * h[k + 8:k + 16]
                        acc[c] = a if acc[c] is None else acc[c] + a
                yield 40
            out["vpu"] = acc

        _interleave(vpu(), mxu())
        return x + b2[...] + _join(out["mxu"]) + _row_sum(_join(out["vpu"]))

    def shared_attention(x):
        y, r = _layernorm(x)
        scale = r * SCORE_SCALE
        p_of, acc_mxu, acc_vpu = {}, [None] * NC, [None] * NC
        never = zero[...] > 0.0
        mxu_trail, vpu_trail, previous_task = [], [], []

        def not_before(trail, lag, value):
            return value if len(trail) < lag else jnp.where(never, trail[-lag], value)

        def lhs(value, lag):
            head, *rest = _cols(value)
            return _join([not_before(vpu_trail, lag, head)] + rest).astype(BF16)

        def paced(values):
            return [not_before(mxu_trail, 6, values[0])] + values[1:]

        def mxu():
            q_of, o_of = {}, {}
            for g in MXU_GROUPS:
                q = None
                for j in range(G):
                    qj = _mm(lhs(y, 24), tiles(T_WQ + (g * G + j) * NC, NC))
                    q = qj if q is None else jnp.where(row == j, qj, q)
                    mxu_trail.append(qj)
                    yield 40 * GUESS_MXU
                q_of[g] = q
            for g in MXU_GROUPS:
                s = None
                for j in range(G):
                    sj = _cols(_mm(lhs(q_of[g], 24), pltpu.bitcast(k_mxu[g * G + j], BF16)))
                    s = sj if s is None else [jnp.where(row == j, a, b) for a, b in zip(sj, s)]
                    mxu_trail.append(sj[-1])
                    yield 64 * GUESS_MXU
                p_of[g] = _softmax(s, scale)
            for g in MXU_GROUPS:
                p, inv = p_of[g]
                o = []
                for j in range(G):
                    o.append(_mm(_join(p).astype(BF16), tiles(T_V + (g * G + j) * NK, NK)))
                    mxu_trail.append(o[-1])
                    yield 64 * GUESS_MXU
                o_of[g] = _join(jnp.where(row == j, o[j] * inv, 0.0) for j in range(G))
            for g in MXU_GROUPS:
                for c in range(NC):
                    a = _mm(lhs(o_of[g], 48), tiles(T_WO + c * H + g * G, G))
                    acc_mxu[c] = a if acc_mxu[c] is None else acc_mxu[c] + a
                    mxu_trail.append(a)
                    yield 64 * GUESS_MXU

        def contract(first, factors, total, second, acc, handover):
            for d in range(DH):
                rows = slice(d * PITCH, d * PITCH + 8)
                value = _lane_sum(total([first(t, rows) * f for t, f in enumerate(paced(factors))]))
                for t in range(len(acc)):
                    a = second(t, rows) * value
                    acc[t] = a if acc[t] is None else acc[t] + a
                if d == handover:
                    previous_task.append(acc[0])
                yield value

        def vpu():
            for i, g in enumerate(VPU_GROUPS):
                s = [None] * NK
                total = (lambda xs: _sum(xs[:2]) + _sum(xs[2:]), _sum)[i]
                for q in contract(lambda c, rows: wq_vpu[i, c, rows, :],
                                  [not_before(previous_task, 1, v) for v in _cols(y)], total,
                                  lambda t, rows: k_vpu[i, t, rows, :], s, (127, 95)[i]):
                    vpu_trail.append((q, s[0])[i])
                    yield 25 * GUESS_VPU
                p_of[g] = _softmax(s, scale)
                yield 20
            for i, g in enumerate(VPU_GROUPS):
                p, inv = p_of[g]
                inv = not_before(previous_task, 1, inv)
                for _ in contract(lambda t, rows: v_vpu[i, t, rows, :],
                                  [t * inv for t in p], functools.partial(_tree, _add),
                                  lambda c, rows: wo_vpu[i, c, rows, :], acc_vpu, 87):
                    vpu_trail.append(acc_vpu[-1])
                    yield 25 * GUESS_VPU

        _interleave(vpu(), mxu())
        return x + _row_sum(_join(a + b for a, b in zip(acc_mxu, acc_vpu)))

    slot = LAST % 2
    pieces, first_head = [], 0
    for i, n in enumerate(LAST_PIECES):
        pieces.append((range(first_head, first_head + n), S_V_LOWER + i))
        first_head += n
    copies = window(1, UPPER, S_V_UPPER)[V_AHEAD:]
    for heads, sem in pieces:
        copies += window(1, heads, sem)
    start_last = functools.partial(start_kv, LAST)
    wait_kv(slot, 0, range(H), S_K)

    @pl.loop(0, 2)
    def _(i):
        for n, g in enumerate((VPU_GROUPS[0] + i, MXU_GROUPS[0] + i)):
            s = None
            for j in range(G):
                step = G * n + j
                share(2 * G * i + step, 4 * G, copies[:-4 * STEP], start_last, (step, 2 * G + step))
                k = kv[2 * slot, g * G + j].T
                sj = _cols(_mm(q_first[LAST, g * G + j].astype(BF16), k))
                s = sj if s is None else [jnp.where(row == j, a, b) for a, b in zip(sj, s)]
                if n:
                    k_mxu[g * G + j] = pltpu.bitcast(k, U32)
                else:
                    put_head(k_vpu, i, j, k)
            p, inv = _softmax(s, SCORE_SCALE)
            probs[g] = _join(p)
            inv_sum[g] = inv

    def upper_values(i, acc):
        g = VPU_GROUPS[0] + i
        p = probs[g].astype(BF16)
        o = []
        for j in range(G):
            share(G * i + j, 2 * G, copies[-4 * STEP:], start_last, (j, G + j))
            v = kv[2 * slot + 1, g * G + j]
            o.append(jnp.where(row == j, _mm(p, v) * inv_sum[g], 0.0))
            put_head(v_vpu, i, j, v.T)
        o = _join(o).astype(BF16)
        return [acc[c] + _mm(o, tiles(T_WO + c * H + g * G, G)) for c in range(NC)]

    wait_kv(slot, 1, UPPER, S_V_UPPER)
    acc = lax.fori_loop(0, 2, upper_values, [jnp.zeros((8, 128), F32)] * NC)
    for heads, sem in pieces:
        wait_kv(slot, 1, heads, sem)
        g = heads[0] // G
        acc = values(slot, heads, _cols(probs[g]), inv_sum[g], acc, keep=True)
    x = x_rows[LAST] + _row_sum(_join(acc))
    x = shared_mlp(shared_attention(shared_mlp(x)))
    out_ref[...] = jnp.where(out_row == LAST, x, result[...]).astype(out_ref.dtype)


@jax.jit
def pallas_interleave_layers__sliding_block_cached__mixer_channel_mlp__decode_kernel(
    A_x: jax.Array,
    A_k_cache: jax.Array,
    A_v_cache: jax.Array,
    A_wq: jax.Array,
    A_wo: jax.Array,
    B_x: jax.Array,
    B_w1: jax.Array,
    B_b1: jax.Array,
    B_w2: jax.Array,
    B_b2: jax.Array,
):
    vmem = pltpu.VMEM
    features = PITCH * DH + PAD
    out = pl.pallas_call(
        _kernel,
        out_shape=jax.ShapeDtypeStruct((B, D), A_x.dtype),
        in_specs=[pl.BlockSpec(memory_space=pltpu.HBM)] * 9,
        out_specs=pl.BlockSpec(memory_space=pltpu.VMEM),
        scratch_shapes=[
            vmem((4, H, W, DH), BF16),
            vmem((D, H * DH), BF16), vmem((H * DH, D), BF16), vmem((F, D), BF16), vmem((F, D), BF16),
            vmem((B, D), BF16), vmem((F,), BF16), vmem((D,), BF16),
            vmem((T_END, 64 + PAD, 128), U32),
            vmem((len(LOWER), DH // 2, W), U32),
            vmem((2, NC, features, 128), F32), vmem((2, NC, features, 128), F32),
            vmem((NC, F - CROSS * 128 + PAD, 128), F32), vmem((NC, CROSS * 128 + PAD, 128), F32),
            vmem((2, NK, features, 128), F32), vmem((2, NK, features, 128), F32),
            vmem((B, 8, D), F32), vmem((B, H, 8, DH), F32), vmem((8, NF * 128), F32), vmem((8, D), F32),
            vmem((NG, 8, W), F32), vmem((NG, 8, 128), F32), vmem((B, D), F32), vmem((8, 128), F32),
            pltpu.SemaphoreType.DMA((6,)),
        ],
        compiler_params=pltpu.CompilerParams(
            vmem_limit_bytes=124 * 1024 * 1024, disable_bounds_checks=True, disable_semaphore_checks=True),
    )(A_x.reshape(B, D), A_k_cache, A_v_cache, A_wq, A_wo, B_w1.T, B_b1, B_w2, B_b2)
    return out.reshape(B, 1, D)
```

```python
import functools

import jax
import jax.numpy as jnp
from jax import lax
import jax.experimental.pallas as pl
import jax.experimental.pallas.tpu as pltpu

B, D, H, DH, SK, F = 8, 640, 32, 128, 4096, 1728
W = min(4096, max(256, SK // 4))
G = 8
NG = H // G
NC = D // 128
NK = W // 128
NF = -(-F // 128)
LAST = B - 1

F32, BF16, U32 = jnp.float32, jnp.bfloat16, jnp.uint32
SCORE_SCALE = DH ** -0.5 * 1.4426950408889634

KEYS_PER_COPY = 64
WEIGHT_ROWS_PER_COPY = 16
PRIORITIES = (0, 1, 1, 1)
STEP = 32
V_AHEAD = 4 * STEP
LAST_PIECES = (8, 5, 3)

MXU_GROUPS, VPU_GROUPS = (0, 1), (2, 3)
LOWER, UPPER = range(H // 2), range(H // 2, H)
CROSS = 7
PITCH = 12
PAD = 8
GUESS_MXU, GUESS_VPU = 1.1, 1.2 / 4

T_WQ = 0
T_WO = T_WQ + H * NC
T_W1 = T_WO + NC * H
T_W2 = T_W1 + NF * NC
T_V = T_W2 + NC * NF
T_END = T_V + len(LOWER) * NK

S_K, S_V_UPPER, S_V_LOWER = 0, 1, 2
S_SMALL, S_WQ, S_W1, S_WO = 2, 3, 4, 5
S_W2 = S_WQ


def _tree(op, xs):
    xs = list(xs)
    while len(xs) > 1:
        xs = [op(xs[i], xs[i + 1]) if i + 1 < len(xs) else xs[i] for i in range(0, len(xs), 2)]
    return xs[0]


def _spread(items, ways=8):
    per = -(-len(items) // ways)
    return [items[i] for r in range(per) for i in range(r, len(items), per)]


def _interleave(*streams):
    clock = [0.0] * len(streams)
    live = list(range(len(streams)))
    while live:
        for i in sorted(live, key=lambda i: clock[i]):
            cost = next(streams[i], False)
            if cost is False:
                live.remove(i)
                break
            if cost is not None:
                clock[i] += cost
                break
            clock[i] = max(clock[i], min((clock[j] for j in live if j != i), default=clock[i]))


def _mm(a, b):
    return jnp.dot(a, b, preferred_element_type=F32)


def _add(a, b):
    return a + b


def _sum(xs):
    return functools.reduce(_add, xs)


def _cols(x):
    return [x[:, c:c + 128] for c in range(0, x.shape[1], 128)]


def _join(xs):
    return jnp.concatenate(list(xs), axis=1)


def _lane_sum(a):
    return jnp.broadcast_to(jnp.sum(a, axis=1, keepdims=True), (8, 128))


def _row_sum(a):
    return jnp.sum(a, axis=0, keepdims=True)


def _mean(x):
    return jnp.broadcast_to(jnp.mean(x, axis=-1, keepdims=True), (x.shape[0], 128))


def _layernorm(x, mean=None):
    d = x - _join([_mean(x) if mean is None else mean] * NC)
    var = jnp.mean(d * d, axis=-1, keepdims=True)
    return d, jnp.broadcast_to(lax.rsqrt(var + 1e-5), (8, 128))


def _gelu(x):
    c = 0.7978845608028654
    return 0.5 * x * (1.0 + jnp.tanh(x * (c + (c * 0.044715) * (x * x))))


def _softmax(s, scale):
    m = jnp.broadcast_to(jnp.max(_tree(jnp.maximum, s), axis=1, keepdims=True), (8, 128))
    p = [jnp.exp2((t - m) * scale) for t in s]
    return p, 1.0 / _lane_sum(_tree(_add, p))


def _kernel(x_hbm, k_hbm, v_hbm, wq_hbm, wo_hbm, w1t_hbm, b1_hbm, w2_hbm, b2_hbm,
            out_ref,
            kv, wq, wo, w1t, w2, x_in, b1_in, b2_in,
            mxu_tiles, k_mxu, wq_vpu, wo_vpu, w1_vpu, w2_vpu, k_vpu, v_vpu,
            x_rows, q_first, b1, b2, wo_mean, w2_mean, probs, inv_sum, result, zero, sems):
    row = lax.broadcasted_iota(jnp.int32, (8, 128), 0)
    out_row = lax.broadcasted_iota(jnp.int32, (8, D), 0)
    started = [0]

    def start(src, dst, sem):
        priority = PRIORITIES[started[0] % len(PRIORITIES)]
        started[0] += 1
        pltpu.make_async_copy(src, dst, sems.at[sem]).start(priority=priority)

    def wait(ref, sem):
        pltpu.make_async_copy(ref, ref, sems.at[sem]).wait()

    def window(which, heads, sem):
        return [(which, h, s, sem) for s in range(0, W, KEYS_PER_COPY) for h in heads]

    def start_kv(b, copies):
        for which, h, s, sem in copies:
            if not isinstance(s, int):
                s = pl.multiple_of(s, KEYS_PER_COPY)
            start((k_hbm, v_hbm)[which].at[b, h, pl.ds(SK - W + s, KEYS_PER_COPY), :],
                  kv.at[2 * (b % 2) + which, h, pl.ds(s, KEYS_PER_COPY), :], sem)

    def wait_kv(slot, which, heads, sem):
        wait(kv.at[2 * slot + which, pl.ds(heads[0], len(heads))], sem)

    def share(i, n, items, action, candidates=None):
        for k in candidates or range(n):
            part = items[len(items) * k // n:len(items) * (k + 1) // n]
            if part:
                pl.when(i == k)(functools.partial(action, part))

    def tiles(first, n):
        return pltpu.bitcast(jnp.concatenate([mxu_tiles[first + k, 0:64, :] for k in range(n)], axis=0), BF16)

    def put_tiles(first, w):
        words = pltpu.bitcast(w, U32)
        for k in range(w.shape[0] // 128):
            mxu_tiles[first + k, 0:64, :] = words[k * 64:(k + 1) * 64]

    def put_head(ref, group, j, w):
        w = w.astype(F32)
        for t, part in enumerate(_cols(w)):
            ref[group, t, pl.ds(j, DH, stride=PITCH), :] = part

    def lanes(i):
        return pl.ds(pl.multiple_of(i * 128, 128), 128)

    def rows_of(src, dst):
        n = WEIGHT_ROWS_PER_COPY
        return _spread([(src.at[pl.ds(r, n), :], dst.at[pl.ds(r, n), :]) for r in range(0, src.shape[0], n)])

    def start_all(sem, copies):
        for src, dst in copies:
            start(src, dst, sem)

    small = [pltpu.make_async_copy(src, dst, sems.at[S_SMALL])
             for src, dst in ((x_hbm, x_in), (b1_hbm, b1_in), (b2_hbm, b2_in))]
    wq_copies = _spread([(wq_hbm.at[pl.ds(r, 8), pl.ds(c, 1024)], wq.at[pl.ds(r, 8), pl.ds(c, 1024)])
                         for r in range(0, D, 8) for c in range(0, H * DH, 1024)])
    start_all(S_WQ, wq_copies[:16])
    for copy in small:
        copy.start()
    start_all(S_WQ, wq_copies[16:])
    start_all(S_W1, rows_of(w1t_hbm, w1t))
    for copy in small:
        copy.wait()
    x0 = x_in[...].astype(F32)
    for n in range(B):
        x_rows[n] = jnp.broadcast_to(x0[n:n + 1, :], (8, D))
    b1[...] = jnp.zeros((8, NF * 128), F32)
    b1[:, 0:F] = jnp.broadcast_to(b1_in[...].astype(F32).reshape(1, F), (8, F))
    b2[...] = jnp.broadcast_to(b2_in[...].astype(F32).reshape(1, D), (8, D))
    result[...] = jnp.zeros((B, D), F32)
    zero[...] = jnp.zeros((8, 128), F32)
    wait(wq, S_WQ)
    y0, r0 = _layernorm(x0)
    y0 = y0.astype(BF16)
    ahead = window(0, range(H), S_K) + window(1, UPPER, S_V_UPPER)[:V_AHEAD]

    @pl.loop(0, G)
    def _(j):
        for m in range(32):
            r = pl.multiple_of((m % 8 * 32 + m // 8 + 4 * j) * WEIGHT_ROWS_PER_COPY, WEIGHT_ROWS_PER_COPY)
            start(wo_hbm.at[pl.ds(r, WEIGHT_ROWS_PER_COPY), :], wo.at[pl.ds(r, WEIGHT_ROWS_PER_COPY), :], S_WO)
        for g in range(NG):
            h = g * G + j
            w = wq[:, lanes(h)]
            put_tiles(T_WQ + h * NC, w)
            q = _mm(y0, w) * r0
            for n in range(B):
                q_first[n, h] = jnp.broadcast_to(q[n:n + 1, :], (8, DH))
            if g in VPU_GROUPS:
                put_head(wq_vpu, g - VPU_GROUPS[0], j, w.T)

    wait(w1t, S_W1)

    @pl.loop(0, 7)
    def _(i):
        share(i, 4, rows_of(w2_hbm, w2), functools.partial(start_all, S_W2))
        share(i - 4, 3, ahead[:4 * STEP], functools.partial(start_kv, 0))
        put_tiles(T_W1 + i * NC, w1t[lanes(i), :].T)

        @pl.when(7 + i < F // 128)
        def _():
            put_tiles(T_W1 + (7 + i) * NC, w1t[lanes(7 + i), :].T)

        @pl.when(i < NC)
        def _():
            w1_vpu[i, 0:F - CROSS * 128, :] = w1t[CROSS * 128:F, lanes(i)].astype(F32)

    put_tiles(T_W1 + (NF - 1) * NC,
              jnp.concatenate([w1t[F // 128 * 128:F, :], jnp.zeros((NF * 128 - F, D), BF16)], axis=0).T)
    wait(wo, S_WO)
    wait(w2, S_W2)

    @pl.loop(0, G)
    def _(j):
        pl.when(j < 6)(lambda: start_kv(0, [(0, h, (4 + 2 * j + m) * KEYS_PER_COPY, S_K)
                                            for m in range(2) for h in range(H)]))
        pl.when(j >= 6)(lambda: start_kv(0, [(1, h, (4 * (j - 6) + m) * KEYS_PER_COPY, S_V_UPPER)
                                             for m in range(4) for h in UPPER]))
        for c in range(NC):
            put_tiles(T_WO + c * H + 4 * j, wo[pl.ds(pl.multiple_of(j * 512, 512), 512), c * 128:(c + 1) * 128])
        for i, g in enumerate(VPU_GROUPS):
            w = wo[lanes(g * G + j), :].astype(F32)
            put_head(wo_vpu, i, j, _join([w, _mean(w)]))
        for g in MXU_GROUPS:
            wo_mean[g, pl.ds(j, 1), :] = _mean(wo[lanes(g * G + j), :].astype(F32)).T[0:1]
        for i in (j, G + j):
            @pl.when(i < F // 128)
            def _():
                w2_mean[i] = _mean(w2[lanes(i), :].astype(F32)).T[0:8]

        @pl.when(j < NC)
        def _():
            put_tiles(T_W2 + j * NF,
                      jnp.concatenate([w2[:, lanes(j)], jnp.zeros((NF * 128 - F, 128), BF16)], axis=0))
            w2_vpu[j, 0:CROSS * 128, :] = w2[0:CROSS * 128, lanes(j)].astype(F32)

    w2_mean[NF - 1] = _mean(jnp.concatenate(
        [w2[F // 128 * 128:F, :].astype(F32), jnp.zeros((NF * 128 - F, D), F32)], axis=0)).T[0:8]

    def scores(slot, g, q, tick):
        s = None
        for j in range(G):
            sj = _cols(lax.dot_general(q(j), kv[2 * slot, g * G + j], (((1,), (1,)), ((), ())),
                                       preferred_element_type=F32))
            s = sj if s is None else [jnp.where(row == j, a, b) for a, b in zip(sj, s)]
            tick(128)
        return s

    def values(slot, heads, p, inv, acc, tick=lambda work: None, keep=False):
        p = _join(p).astype(BF16)
        o = []
        for h in heads:
            v = kv[2 * slot + 1, h]
            o.append(jnp.where(row == h % G, _mm(p, v) * inv, 0.0))
            if keep:
                put_tiles(T_V + h * NK, v)
            tick(64)
        o = _join(o).astype(BF16)
        out = []
        for c in range(NC):
            out.append(_mm(o, tiles(T_WO + c * H + heads[0], len(heads))))
            tick(8 * len(heads))
        return (out if acc is None else [a + b for a, b in zip(acc, out)]), o

    def mlp(x, tick):
        y, r = _layernorm(x)
        y = y.astype(BF16)
        hidden = []
        for i in range(NF):
            hidden.append(_gelu(_mm(y, tiles(T_W1 + i * NC, NC)) * r + b1[:, i * 128:(i + 1) * 128]))
            tick(40)
        hidden = _join(hidden).astype(BF16)
        out = []
        for c in range(NC):
            out.append(_mm(hidden, tiles(T_W2 + c * NF, NF)))
            tick(8 * NF)
        return x + b2[...] + _join(out)

    @pl.loop(0, LAST)
    def _(b):
        slot = b % 2
        upper, lower = window(1, UPPER, S_V_UPPER)[V_AHEAD:], window(1, LOWER, S_V_LOWER)
        todo = []
        for i in range(0, len(lower), H // 2):
            todo += [(b, c) for c in lower[i:i + H // 2] + upper[i:i + H // 2]]
        v_end = len(todo)
        todo += [(b + 1, c) for c in ahead]
        done = [0]

        def ticker(end, work):
            begin, seen = done[0], [0]

            def tick(n):
                seen[0] += n
                while done[0] < begin + (end - begin) * seen[0] // work:
                    start_kv(todo[done[0]][0], [todo[done[0]][1]])
                    done[0] += 1
            return tick

        group = lambda g: range(g * G, (g + 1) * G)
        wait_kv(slot, 0, range(H), S_K)
        tick = ticker(v_end - 2 * STEP, H * 128)
        for g in range(NG):
            p, inv = _softmax(scores(slot, g, lambda j: q_first[b, g * G + j].astype(BF16), tick), SCORE_SCALE)
            probs[g] = _join(p)
            inv_sum[g] = inv
        wait_kv(slot, 1, UPPER, S_V_UPPER)
        acc = None
        tick = ticker(v_end + 2 * STEP, len(UPPER) * 104)
        for g in VPU_GROUPS:
            acc, _ = values(slot, group(g), _cols(probs[g]), inv_sum[g], acc, tick)
        wait_kv(slot, 1, LOWER, S_V_LOWER)
        tick = ticker(len(todo), len(LOWER) * 104 + 2 * 80 * NF + H * 272)
        for g in MXU_GROUPS:
            acc, _ = values(slot, group(g), _cols(probs[g]), inv_sum[g], acc, tick)
        x = mlp(x_rows[b] + _row_sum(_join(acc)), tick)

        y, r = _layernorm(x)
        y = y.astype(BF16)
        acc = None
        for g in range(NG):
            q = []
            for h in group(g):
                q.append(_mm(y, tiles(T_WQ + h * NC, NC)).astype(BF16))
                tick(40)
            p, inv = _softmax(scores(slot, g, lambda j: q[j], tick), r * SCORE_SCALE)
            acc, _ = values(slot, group(g), p, inv, acc, tick)
        x = mlp(x + _row_sum(_join(acc)), tick)
        assert done[0] == len(todo)
        result[...] = jnp.where(out_row == b, x, result[...])

    def wo_share(g, o):
        return _row_sum(_lane_sum(_sum(_cols(o.astype(F32))) * wo_mean[g]))

    def shared_mlp(x, mean):
        y, r = _layernorm(x, mean)
        y_mxu, y_vpu = y.astype(BF16), _cols(y)
        hidden, out = {}, {}
        width = lambda i: min(128, F - i * 128)

        def activate(i, h):
            n = width(i)
            hidden[i] = _gelu(h * r[:, 0:n] + b1[:, i * 128:i * 128 + n])

        def mxu():
            for i in range(CROSS):
                activate(i, _mm(y_mxu, tiles(T_W1 + i * NC, NC)))
                yield 40 * GUESS_MXU
            acc = [None] * NC
            for i in range(CROSS, NF):
                while i not in hidden:
                    yield None
                h = hidden[i].astype(BF16)
                for c in range(NC):
                    a = _mm(h, pltpu.bitcast(mxu_tiles[T_W2 + c * NF + i, 0:width(i) // 2, :], BF16))
                    acc[c] = a if acc[c] is None else acc[c] + a
                yield width(i) / 128 * 40 * GUESS_MXU
            out["mxu"] = acc

        def vpu():
            for i in range(CROSS, NF):
                first = (i - CROSS) * 128
                parts = [_sum([w1_vpu[c, f:f + 8, :] * y_vpu[c] for c in range(NC)])
                         for f in range(first, first + width(i), 8)]
                parts = jnp.concatenate(parts, axis=0).T
                h = _row_sum(_sum([parts[k:k + 8] for k in range(0, 128, 8)]))
                activate(i, jnp.broadcast_to(h, (8, width(i))))
                yield width(i) / 128 * 43
            acc = [None] * NC
            for i in range(CROSS):
                while i not in hidden:
                    yield None
                h = jnp.concatenate([hidden[i]] * 16, axis=0).astype(BF16).T.astype(F32)
                for k in range(0, 128, 16):
                    f = i * 128 + k
                    for c in range(NC):
                        a = w2_vpu[c, f:f + 8, :] * h[k:k + 8] + w2_vpu[c, f + 8:f + 16, :] * h[k + 8:k + 16]
                        acc[c] = a if acc[c] is None else acc[c] + a
                yield 40
            out["vpu"] = acc

        _interleave(vpu(), mxu())
        h = [hidden[i].astype(BF16).astype(F32) for i in range(NF)]
        h[-1] = _join([h[-1], jnp.zeros((8, NF * 128 - F), F32)])
        mean = mean + _mean(b2[...]) + _lane_sum(_sum([h[i] * w2_mean[i] for i in range(NF)]))
        return x + b2[...] + _join(out["mxu"]) + _row_sum(_join(out["vpu"])), mean

    def shared_attention(x, mean):
        y, r = _layernorm(x, mean)
        scale = r * SCORE_SCALE
        p_of, o_of, acc_mxu, acc_vpu = {}, {}, [None] * NC, [None] * NC
        never = zero[...] > 0.0
        mxu_trail, vpu_trail, previous_task = [], [], []

        def not_before(trail, lag, value):
            return value if len(trail) < lag else jnp.where(never, trail[-lag], value)

        def paced(values):
            return [not_before(mxu_trail, 6 if previous_task else 5, values[0])] + values[1:]

        def mxu():
            q_of = {}
            for g in MXU_GROUPS:
                q = None
                for j in range(G):
                    qj = _mm(y.astype(BF16), tiles(T_WQ + (g * G + j) * NC, NC))
                    q = qj if q is None else jnp.where(row == j, qj, q)
                    mxu_trail.append(qj)
                    yield 40 * GUESS_MXU
                q_of[g] = q
            for g in MXU_GROUPS:
                s = None
                for j in range(G):
                    q = not_before(vpu_trail, 20, q_of[g]).astype(BF16)
                    sj = _cols(_mm(q, pltpu.bitcast(k_mxu[g * G + j], BF16)))
                    s = sj if s is None else [jnp.where(row == j, a, b) for a, b in zip(sj, s)]
                    mxu_trail.append(sj[-1])
                    yield 64 * GUESS_MXU
                p_of[g] = _softmax(s, scale)
            for g in MXU_GROUPS:
                p, inv = p_of[g]
                o = []
                for j in range(G):
                    o.append(_mm(_join(p).astype(BF16), tiles(T_V + (g * G + j) * NK, NK)))
                    mxu_trail.append(o[-1])
                    yield 64 * GUESS_MXU
                o_of[g] = _join(jnp.where(row == j, o[j] * inv, 0.0) for j in range(G)).astype(BF16)
            for g in MXU_GROUPS:
                for c in range(NC):
                    a = _mm(o_of[g], tiles(T_WO + c * H + g * G, G))
                    acc_mxu[c] = a if acc_mxu[c] is None else acc_mxu[c] + a
                    mxu_trail.append(a)
                    yield 64 * GUESS_MXU

        def contract(first, factors, total, second, acc, handover):
            for d in range(DH):
                rows = slice(d * PITCH, d * PITCH + 8)
                value = _lane_sum(total([first(t, rows) * f for t, f in enumerate(paced(factors))]))
                for t in range(len(acc)):
                    a = second(t, rows) * value
                    acc[t] = a if acc[t] is None else acc[t] + a
                if d == handover:
                    previous_task.append(acc[0])
                yield value

        def vpu():
            for i, g in enumerate(VPU_GROUPS):
                s = [None] * NK
                total = (lambda xs: _sum(xs[:2]) + _sum(xs[2:]), _sum)[i]
                for q in contract(lambda c, rows: wq_vpu[i, c, rows, :],
                                  [not_before(previous_task, 1, v) for v in _cols(y)], total,
                                  lambda t, rows: k_vpu[i, t, rows, :], s, (127, 79)[i]):
                    vpu_trail.append((q, s[0])[i])
                    yield 25 * GUESS_VPU
                p_of[g] = _softmax(s, scale)
                yield 20
            for i, g in enumerate(VPU_GROUPS):
                p, inv = p_of[g]
                inv = not_before(previous_task, 1, inv)
                steps = contract(lambda t, rows: v_vpu[i, t, rows, :],
                                 [t * inv for t in p], functools.partial(_tree, _add),
                                 lambda c, rows: wo_vpu[i, c, rows, :], acc_vpu, 87)
                for d, _ in enumerate(steps):
                    if g == VPU_GROUPS[-1] and d == 95:
                        acc_vpu.append(_mean(_join(acc_vpu)))
                    yield 25 * GUESS_VPU

        _interleave(vpu(), mxu())
        mean = mean + _sum([wo_share(g, o_of[g]) for g in MXU_GROUPS]) + _row_sum(acc_vpu[NC])
        return x + _row_sum(_join(a + b for a, b in zip(acc_mxu, acc_vpu))), mean

    slot = LAST % 2
    pieces, first_head = [], 0
    for i, n in enumerate(LAST_PIECES):
        pieces.append((range(first_head, first_head + n), S_V_LOWER + i))
        first_head += n
    copies = window(1, UPPER, S_V_UPPER)[V_AHEAD:]
    for heads, sem in pieces:
        copies += window(1, heads, sem)
    start_last = functools.partial(start_kv, LAST)
    wait_kv(slot, 0, range(H), S_K)

    @pl.loop(0, 2)
    def _(i):
        for n, g in enumerate((VPU_GROUPS[0] + i, MXU_GROUPS[0] + i)):
            s = None
            for j in range(G):
                step = G * n + j
                share(2 * G * i + step, 4 * G, copies[:-4 * STEP], start_last, (step, 2 * G + step))
                k = kv[2 * slot, g * G + j].T
                sj = _cols(_mm(q_first[LAST, g * G + j].astype(BF16), k))
                s = sj if s is None else [jnp.where(row == j, a, b) for a, b in zip(sj, s)]
                if n:
                    k_mxu[g * G + j] = pltpu.bitcast(k, U32)
                else:
                    put_head(k_vpu, i, j, k)
            p, inv = _softmax(s, SCORE_SCALE)
            probs[g] = _join(p)
            inv_sum[g] = inv

    def upper_values(i, acc):
        g = VPU_GROUPS[0] + i
        p = probs[g].astype(BF16)
        o = []
        for j in range(G):
            share(G * i + j, 2 * G, copies[-4 * STEP:], start_last, (j, G + j))
            v = kv[2 * slot + 1, g * G + j]
            o.append(jnp.where(row == j, _mm(p, v) * inv_sum[g], 0.0))
            put_head(v_vpu, i, j, v.T)
        o = _join(o).astype(BF16)
        return [acc[c] + _mm(o, tiles(T_WO + c * H + g * G, G)) for c in range(NC)]

    wait_kv(slot, 1, UPPER, S_V_UPPER)
    acc = lax.fori_loop(0, 2, upper_values, [jnp.zeros((8, 128), F32)] * NC)
    for heads, sem in pieces:
        wait_kv(slot, 1, heads, sem)
        g = heads[0] // G
        before = acc
        acc, o = values(slot, heads, _cols(probs[g]), inv_sum[g], acc, keep=True)
    mean = _mean(x_rows[LAST] + _row_sum(_join(before))) + wo_share(g, o)
    x = x_rows[LAST] + _row_sum(_join(acc))
    x, _ = shared_mlp(*shared_attention(*shared_mlp(x, mean)))
    out_ref[...] = jnp.where(out_row == LAST, x, result[...]).astype(out_ref.dtype)


@jax.jit
def pallas_interleave_layers__sliding_block_cached__mixer_channel_mlp__decode_kernel(
    A_x: jax.Array,
    A_k_cache: jax.Array,
    A_v_cache: jax.Array,
    A_wq: jax.Array,
    A_wo: jax.Array,
    B_x: jax.Array,
    B_w1: jax.Array,
    B_b1: jax.Array,
    B_w2: jax.Array,
    B_b2: jax.Array,
):
    vmem = pltpu.VMEM
    features = PITCH * DH + PAD
    out = pl.pallas_call(
        _kernel,
        out_shape=jax.ShapeDtypeStruct((B, D), A_x.dtype),
        in_specs=[pl.BlockSpec(memory_space=pltpu.HBM)] * 9,
        out_specs=pl.BlockSpec(memory_space=pltpu.VMEM),
        scratch_shapes=[
            vmem((4, H, W, DH), BF16),
            vmem((D, H * DH), BF16), vmem((H * DH, D), BF16), vmem((F, D), BF16), vmem((F, D), BF16),
            vmem((B, D), BF16), vmem((F,), BF16), vmem((D,), BF16),
            vmem((T_END, 64 + PAD, 128), U32),
            vmem((len(LOWER), DH // 2, W), U32),
            vmem((2, NC, features, 128), F32), vmem((2, NC + 1, features, 128), F32),
            vmem((NC, F - CROSS * 128 + PAD, 128), F32), vmem((NC, CROSS * 128 + PAD, 128), F32),
            vmem((2, NK, features, 128), F32), vmem((2, NK, features, 128), F32),
            vmem((B, 8, D), F32), vmem((B, H, 8, DH), F32), vmem((8, NF * 128), F32), vmem((8, D), F32),
            vmem((len(MXU_GROUPS), G, DH), F32), vmem((NF, 8, 128), F32),
            vmem((NG, 8, W), F32), vmem((NG, 8, 128), F32), vmem((B, D), F32), vmem((8, 128), F32),
            pltpu.SemaphoreType.DMA((6,)),
        ],
        compiler_params=pltpu.CompilerParams(
            vmem_limit_bytes=124 * 1024 * 1024, disable_bounds_checks=True, disable_semaphore_checks=True),
    )(A_x.reshape(B, D), A_k_cache, A_v_cache, A_wq, A_wo, B_w1.T, B_b1, B_w2, B_b2)
    return out.reshape(B, 1, D)
```
